```python
import jax
import jax.numpy as jnp

def _softmax(x, axis=-1):
    return jax.nn.softmax(x, axis=axis)

def _gelu(x):
    return jax.nn.gelu(x, approximate=True)

def _silu(x):
    return jax.nn.silu(x)

def _sigmoid(x):
    return jax.nn.sigmoid(x)

def _layernorm(x, axis=-1, eps=1e-05):
    m = jnp.mean(x, axis=axis, keepdims=True)
    v = jnp.var(x, axis=axis, keepdims=True)
    return (x - m) / jnp.sqrt(v + eps)

def _scatter_add(tgt, idx, src, axis=0):
    return tgt.at[idx].add(src)

def _segment_sum(src, seg, n):
    return jax.ops.segment_sum(src, seg, n)

class _Rng:

    def __init__(self, key):
        self._k = key

    def _next(self):
        self._k, sub = jax.random.split(self._k)
        return sub

    def normal(self, shape):
        return jax.random.normal(self._next(), shape, dtype=jnp.bfloat16)

    def randint(self, lo, hi, shape):
        return jax.random.randint(self._next(), shape, lo, hi, dtype=jnp.int32)

    def uniform(self, shape, lo=0.0, hi=1.0):
        return jax.random.uniform(self._next(), shape, jnp.bfloat16, lo, hi)

    def permutation(self, n):
        return jax.random.permutation(self._next(), n)
kernel_name = 'adaLN_cond__compressed_kv_cla__mixer_s_mlp__prompt'

def setup_inputs():
    _rng = _Rng(jax.random.key(int.from_bytes(__import__("os").urandom(4), "little")))
    _w = lambda a: (lambda t: t.astype(jnp.bfloat16) if jnp.issubdtype(t.dtype, jnp.floating) else t)(jnp.asarray(a))

    def _A_setup():
        B, H, Sq, Sk, D, M = (1, 32, 2048, 2048, 128, 640)
        Dc = 4 * D
        return {'x': _w((lambda *s: _rng.normal(s) * 0.05)(B, Sq, M)), 'c_kv': _w((lambda *s: _rng.normal(s) * 0.05)(B, Sk, Dc)), 'w_q': _w((lambda *s: _rng.normal(s) * 0.05)(M, H, D) * M ** (-0.5)), 'w_uk': _w((lambda *s: _rng.normal(s) * 0.05)(Dc, H, D) * Dc ** (-0.5)), 'w_uv': _w((lambda *s: _rng.normal(s) * 0.05)(Dc, H, D) * Dc ** (-0.5)), 'w_o': _w((lambda *s: _rng.normal(s) * 0.05)(H, D, M) * (H * D) ** (-0.5))}
    _A_in = _A_setup()

    def _B_setup():
        B, S, D, F = (1, 2048, 640, 1728)
        return {'x': _w((lambda *s: _rng.normal(s) * 0.05)(B, S, D)), 'w1': _w((lambda *s: _rng.normal(s) * 0.05)(D, D) * D ** (-0.5)), 'w2': _w((lambda *s: _rng.normal(s) * 0.05)(D, D) * D ** (-0.5)), 'w3': _w((lambda *s: _rng.normal(s) * 0.05)(D, F) * D ** (-0.5)), 'w4': _w((lambda *s: _rng.normal(s) * 0.05)(F, D) * F ** (-0.5))}
    _B_in = _B_setup()
    return {'A_x': _A_in['x'], 'A_c_kv': _A_in['c_kv'], 'A_w_q': _A_in['w_q'], 'A_w_uk': _A_in['w_uk'], 'A_w_uv': _A_in['w_uv'], 'A_w_o': _A_in['w_o'], 'B_x': _B_in['x'], 'B_w1': _B_in['w1'], 'B_w2': _B_in['w2'], 'B_w3': _B_in['w3'], 'B_w4': _B_in['w4'], 'c': _w((lambda *s: _rng.normal(s) * 0.05)(1, 640)), 'w_mod': _w((lambda *s: _rng.normal(s) * 0.05)(640, 6 * 640) * 640 ** (-0.5))}

def reference(A_x, A_c_kv, A_w_q, A_w_uk, A_w_uv, A_w_o, B_x, B_w1, B_w2, B_w3, B_w4, c, w_mod):

    def _A_ref(x, c_kv, w_q, w_uk, w_uv, w_o):
        B, Sq, M = (x.shape[0], x.shape[1], x.shape[2])
        Sk = c_kv.shape[1]
        H, D = (w_q.shape[1], w_q.shape[2])
        q = jnp.einsum('bqm,mhd->bhqd', x, w_q)
        k = jnp.einsum('bkc,chd->bhkd', c_kv, w_uk)
        v = jnp.einsum('bkc,chd->bhkd', c_kv, w_uv)
        scores = jnp.einsum('bhqd,bhkd->bhqk', q, k) * D ** (-0.5)
        off = Sk - Sq
        qi = jnp.arange(Sq)[:, None]
        kj = jnp.arange(Sk)[None, :]
        cmask = kj <= qi + off
        scores = jnp.where(cmask[None, None], scores, -1000000000.0)
        p = _softmax(scores, axis=-1)
        ctx = jnp.einsum('bhqk,bhkd->bhqd', p, v)
        return jnp.einsum('bhqd,hdm->bqm', ctx, w_o)

    def _B_ref(x, w1, w2, w3, w4):
        B, S, D = x.shape
        h = _gelu(_layernorm(x, axis=-1) @ w1)
        c = D // 4
        g0 = jnp.pad(h[:, :, 0 * c:1 * c], ((0, 0), (1, 0), (0, 0)))[:, :S, :]
        g1 = jnp.pad(h[:, :, 1 * c:2 * c], ((0, 0), (0, 1), (0, 0)))[:, 1:, :]
        g2 = jnp.pad(h[:, :, 2 * c:3 * c], ((0, 0), (2, 0), (0, 0)))[:, :S, :]
        g3 = jnp.pad(h[:, :, 3 * c:], ((0, 0), (0, 2), (0, 0)))[:, 2:, :]
        hs = jnp.concatenate([g0, g1, g2, g3], axis=-1) @ w2
        x1 = x + hs
        h2 = _gelu(_layernorm(x1, axis=-1) @ w3) @ w4
        return x1 + h2
    x = A_x
    mod = (_silu(c) @ w_mod).reshape(c.shape[0], 6, 1, -1)
    sa, ca, ga, sb, cb, gb = (mod[:, 0].copy(), mod[:, 1].copy(), mod[:, 2].copy(), mod[:, 3].copy(), mod[:, 4].copy(), mod[:, 5].copy())
    h = _layernorm(x, axis=-1) * (1 + ca) + sa
    x = x + ga * _A_ref(h, A_c_kv, A_w_q, A_w_uk, A_w_uv, A_w_o)
    h = _layernorm(x, axis=-1) * (1 + cb) + sb
    x = x + gb * _B_ref(h, B_w1, B_w2, B_w3, B_w4)
    return x
```

```python
import functools
import math

import jax
import jax.numpy as jnp
import numpy as np
from jax import lax
from jax.experimental import pallas as pl
from jax.experimental.pallas import tpu as pltpu

S = 2048
M = 640
H = 32
D = 128
DC = 512
F = 1728
G = 4
NG = H // G
R = 128
TC = 256
EPS = 1e-5
NEG = -1e9
QSCALE = float(D ** -0.5 * math.log2(math.e))

f32 = jnp.float32
bf16 = jnp.bfloat16
_NT = (((1,), (1,)), ((), ()))


def _dot(a, b):
    return jnp.dot(a, b, preferred_element_type=f32)


def _recip(x):
    r = pltpu.reciprocal(x, approx=True)
    r = r * (2.0 - x * r)
    return r * (2.0 - x * r)


def _layernorm(x):
    mu = jnp.mean(x, axis=-1, keepdims=True)
    xc = x - mu
    var = jnp.mean(xc * xc, axis=-1, keepdims=True)
    return xc * lax.rsqrt(var + EPS)


def _gelu(x):
    c = math.sqrt(2.0 / math.pi)
    return 0.5 * x * (1.0 + jnp.tanh(c * (x + 0.044715 * (x * x * x))))


def _relayout(w_raw, half, kdim, pair, dst_ref):
    w = w_raw.at[half].reshape(kdim * 8, D)
    for p in range(G // 2):
        x = w[pl.ds(pair + p, kdim, stride=8), :]
        lo = pltpu.bitcast(x << 16, f32).astype(bf16)
        hi = pltpu.bitcast(x & jnp.uint32(0xFFFF0000), f32).astype(bf16)
        dst_ref[:, (2 * p) * D:(2 * p + 1) * D] = lo
        dst_ref[:, (2 * p + 1) * D:(2 * p + 2) * D] = hi


def _attention_group(g, q_s, k_s, v_s, ctx_s):
    nstrip = S // R
    items = [(u, i) for u in range(G) for i in range(nstrip - 1, -1, -1)]
    n = len(items)
    LA = 2
    st = {}
    row = lax.broadcasted_iota(jnp.int32, (R, R), 0)
    col = lax.broadcasted_iota(jnp.int32, (R, R), 1)
    causal = col <= row

    def scores(t):
        u, i = items[t]
        e = (i + 1) * R
        q = q_s[i * R:(i + 1) * R, u * D:(u + 1) * D]
        s = lax.dot_general(q, k_s[0:e, u * D:(u + 1) * D], _NT, preferred_element_type=f32)
        tiles = [s[:, j * 128:(j + 1) * 128] for j in range(i)]
        tiles.append(jnp.where(causal, s[:, e - R:e], NEG))
        st[t] = {"tiles": tiles}

    def rowmax(t):
        d = st[t]
        m = d["tiles"][0]
        for x in d["tiles"][1:]:
            m = jnp.maximum(m, x)
        d["m"] = jnp.max(m, axis=1, keepdims=True)

    def pv(t):
        u, i = items[t]
        d = st[t]
        e = (i + 1) * R
        ps = [jnp.exp2(x - d["m"]) for x in d["tiles"]]
        l = ps[0]
        for x in ps[1:]:
            l = l + x
        d["l"] = l
        p = jnp.concatenate(ps, axis=1).astype(bf16)
        d["o"] = _dot(p, v_s[0:e, u * D:(u + 1) * D])

    def finish(t):
        u, i = items[t]
        d = st.pop(t)
        lrow = jnp.sum(d["l"], axis=1, keepdims=True)
        ctx_s[g, i * R:(i + 1) * R, u * D:(u + 1) * D] = (d["o"] * _recip(lrow)).astype(bf16)

    for t in range(-LA, n + 1):
        if 0 <= t + LA < n:
            scores(t + LA)
        if 0 <= t + LA - 1 < n:
            rowmax(t + LA - 1)
        if 0 <= t < n:
            pv(t)
        if 0 <= t - 1 < n:
            finish(t - 1)


def _tail(x_s, ctx_s, wo_s, w1_s, w2_s, w3_s, w4_s, c_s, wmod_s, h1_s, out_s, o_hbm, osem):
    n = S // TC
    st = {}
    mod = _modulation(c_s, wmod_s[...])
    ga = mod[:, 0:M]
    sb = mod[:, M:2 * M]
    cb1 = 1.0 + mod[:, 2 * M:3 * M]
    gb = mod[:, 3 * M:4 * M]
    lane = lax.broadcasted_iota(jnp.int32, (1, 128), 1)
    out_copies = []

    def rows(t):
        return slice(t * TC, (t + 1) * TC)

    def oproj(t):
        acc = _dot(ctx_s[0, rows(t), :], wo_s[0:G * D, :])
        for g in range(1, NG):
            acc = acc + _dot(ctx_s[g, rows(t), :], wo_s[g * G * D:(g + 1) * G * D, :])
        x1 = x_s[rows(t), :].astype(f32) + ga * acc
        h = _layernorm(x1) * cb1 + sb
        st[t] = {"x1": x1, "h": h, "n1": _layernorm(h).astype(bf16)}

    def mm1(t):
        d = st[t]
        h1_s[8 + t * TC:8 + (t + 1) * TC, :] = _gelu(_dot(d.pop("n1"), w1_s[...]))

    def mm2(t):
        d = st[t]
        r0 = 8 + t * TC

        def ld(shift, tile):
            return h1_s[r0 + shift:r0 + shift + TC, tile * 128:(tile + 1) * 128]

        c = M // 4
        g = jnp.concatenate([
            ld(-1, 0),
            jnp.where(lane < c - 128, ld(-1, 1), ld(1, 1)),
            jnp.where(lane < 2 * c - 256, ld(1, 2), ld(-2, 2)),
            jnp.where(lane < 3 * c - 384, ld(-2, 3), ld(2, 3)),
            ld(2, 4),
        ], axis=1).astype(bf16)
        u = d.pop("h") + _dot(g, w2_s[...])
        d["u"] = u
        d["n2"] = _layernorm(u).astype(bf16)

    def mm3(t):
        d = st[t]
        a = lax.dot_general(d.pop("n2"), w3_s[...], _NT, preferred_element_type=f32)
        d["a"] = _gelu(a).astype(bf16)

    def mm4(t):
        d = st.pop(t)
        y = d["u"] + _dot(d["a"], w4_s[...])
        out_s[rows(t), :] = (d["x1"] + gb * y).astype(out_s.dtype)
        cp = pltpu.make_async_copy(out_s.at[rows(t), :], o_hbm.at[rows(t), :], osem.at[t])
        cp.start()
        out_copies.append(cp)

    for t in range(-2, n + 1):
        if 0 <= t + 2 < n:
            oproj(t + 2)
        if 0 <= t - 1 < n:
            mm3(t - 1)
        if 0 <= t + 1 < n:
            mm1(t + 1)
        if 0 <= t - 1 < n:
            mm4(t - 1)
        if 0 <= t < n:
            mm2(t)
    for cp in out_copies:
        cp.wait()


def _modulation(c_s, wmod):
    cv = c_s[...].astype(f32)
    sc = (cv * jax.nn.sigmoid(cv)).astype(bf16)
    return _dot(jnp.broadcast_to(sc, (16, M)), wmod)[0:1]


def _kernel(x_hbm, ckv_hbm, wq_hbm, wk_hbm, wv_hbm, wo_hbm, w1_hbm, w2_hbm, w3_hbm, w4_hbm, c_hbm, wmod_hbm,
            o_hbm,
            x_s, ckv_s, wq_raw, wk_raw, wv_raw, wo_s, w1_s, w2_s, w3_s, w4_s, c_s, wmod_a, wmod_b,
            h_s, wq_s, wk_s, wv_s, q_s, k_s, v_s, ctx_s, h1_s, out_s, sems, osem):
    wq32, wk32, wv32 = (w.bitcast(jnp.uint32) for w in (wq_hbm, wk_hbm, wv_hbm))
    hp = H // 4
    moves = [
        (ckv_hbm, ckv_s),
        (wk32.at[:, 0:hp, :], wk_raw.at[0]),
        (wv32.at[:, 0:hp, :], wv_raw.at[0]),
        (x_hbm, x_s),
        (c_hbm, c_s),
        (wmod_hbm.at[:, 0:2 * M], wmod_a),
        (wq32.at[:, 0:hp, :], wq_raw.at[0]),
        (wk32.at[:, hp:2 * hp, :], wk_raw.at[1]),
        (wv32.at[:, hp:2 * hp, :], wv_raw.at[1]),
        (wq32.at[:, hp:2 * hp, :], wq_raw.at[1]),
        (wo_hbm, wo_s),
        (wmod_hbm.at[:, 2 * M:6 * M], wmod_b),
        (w1_hbm, w1_s),
        (w2_hbm, w2_s),
        (w3_hbm, w3_s),
        (w4_hbm, w4_s),
    ]
    copies = [pltpu.make_async_copy(src, dst, sems.at[i]) for i, (src, dst) in enumerate(moves)]
    for cp in copies:
        cp.start()
    (cp_ckv, cp_wk0, cp_wv0, cp_x, cp_c, cp_wma, cp_wq0, cp_wk1, cp_wv1, cp_wq1) = copies[:10]

    def k_proj(half, pair):
        _relayout(wk_raw, half, DC, pair, wk_s)
        k_s[...] = _dot(ckv_s[...], wk_s[...]).astype(bf16)

    def v_proj(half, pair):
        _relayout(wv_raw, half, DC, pair, wv_s)
        v_s[...] = _dot(ckv_s[...], wv_s[...]).astype(bf16)

    def q_proj(half, pair):
        _relayout(wq_raw, half, M, pair, wq_s)
        q_s[...] = (_dot(h_s[...], wq_s[...]) * QSCALE).astype(bf16)

    h1_s[0:8, :] = jnp.zeros((8, M), f32)
    h1_s[8 + S:16 + S, :] = jnp.zeros((8, M), f32)

    cp_ckv.wait()
    cp_wk0.wait()
    k_proj(0, 0)
    cp_wv0.wait()
    v_proj(0, 0)
    cp_x.wait()
    cp_c.wait()
    cp_wma.wait()
    mod = _modulation(c_s, wmod_a[...])
    sa = mod[:, 0:M]
    ca1 = 1.0 + mod[:, M:2 * M]
    LC = 256

    def ln_chunk(i):
        xi = x_s[i * LC:(i + 1) * LC, :].astype(f32)
        h_s[i * LC:(i + 1) * LC, :] = (_layernorm(xi) * ca1 + sa).astype(bf16)

    ln_chunk(0)
    ln_chunk(1)
    cp_wq0.wait()
    _relayout(wq_raw, 0, M, 0, wq_s)
    for i in range(S // LC):
        if i + 2 < S // LC:
            ln_chunk(i + 2)
        rs = slice(i * LC, (i + 1) * LC)
        q_s[rs, :] = (_dot(h_s[rs, :], wq_s[...]) * QSCALE).astype(bf16)

    def group(g, carry):
        @pl.when(g == 1)
        def _():
            cp_wk1.wait()
            cp_wv1.wait()
            cp_wq1.wait()

        _attention_group(g, q_s, k_s, v_s, ctx_s)

        @pl.when(g < NG - 1)
        def _():
            half = (g + 1) // (NG // 2)
            pair = ((g + 1) % (NG // 2)) * (G // 2)
            k_proj(half, pair)
            q_proj(half, pair)
            v_proj(half, pair)

        return carry

    lax.fori_loop(0, NG, group, 0)

    for cp in copies[10:]:
        cp.wait()
    _tail(x_s, ctx_s, wo_s, w1_s, w2_s, w3_s, w4_s, c_s, wmod_b, h1_s, out_s, o_hbm, osem)


@jax.jit
def pallas_adaLN_cond__compressed_kv_cla__mixer_s_mlp__prompt_kernel(
    A_x: jax.Array,
    A_c_kv: jax.Array,
    A_w_q: jax.Array,
    A_w_uk: jax.Array,
    A_w_uv: jax.Array,
    A_w_o: jax.Array,
    B_x: jax.Array,
    B_w1: jax.Array,
    B_w2: jax.Array,
    B_w3: jax.Array,
    B_w4: jax.Array,
    c: jax.Array,
    w_mod: jax.Array,
):
    del B_x
    x = A_x.reshape(S, M)
    ckv = A_c_kv.reshape(S, DC)
    wo = A_w_o.reshape(H * D, M)

    any_spec = pl.BlockSpec(memory_space=pl.ANY)
    scratch = [
        pltpu.VMEM((S, M), bf16),
        pltpu.VMEM((S, DC), bf16),
        pltpu.VMEM((2, M, 8, D), jnp.uint32),
        pltpu.VMEM((2, DC, 8, D), jnp.uint32),
        pltpu.VMEM((2, DC, 8, D), jnp.uint32),
        pltpu.VMEM((H * D, M), bf16),
        pltpu.VMEM((M, M), bf16),
        pltpu.VMEM((M, M), bf16),
        pltpu.VMEM((F, M), bf16),
        pltpu.VMEM((F, M), bf16),
        pltpu.VMEM((1, M), bf16),
        pltpu.VMEM((M, 2 * M), bf16),
        pltpu.VMEM((M, 4 * M), bf16),
        pltpu.VMEM((S, M), bf16),
        pltpu.VMEM((M, G * D), bf16),
        pltpu.VMEM((DC, G * D), bf16),
        pltpu.VMEM((DC, G * D), bf16),
        pltpu.VMEM((S, G * D), bf16),
        pltpu.VMEM((S, G * D), bf16),
        pltpu.VMEM((S, G * D), bf16),
        pltpu.VMEM((NG, S, G * D), bf16),
        pltpu.VMEM((S + 16, M), f32),
        pltpu.VMEM((S, M), bf16),
        pltpu.SemaphoreType.DMA((16,)),
        pltpu.SemaphoreType.DMA((S // TC,)),
    ]
    out = pl.pallas_call(
        _kernel,
        out_shape=jax.ShapeDtypeStruct((S, M), A_x.dtype),
        in_specs=[any_spec] * 12,
        out_specs=any_spec,
        scratch_shapes=scratch,
        compiler_params=pltpu.CompilerParams(vmem_limit_bytes=120 * 1024 * 1024),
    )(x, ckv, A_w_q, A_w_uk, A_w_uv, wo, B_w1, B_w2, B_w3.T, B_w4, c, w_mod)
    return out.reshape(1, S, M)
```

```python
import functools
import math

import jax
import jax.numpy as jnp
import numpy as np
from jax import lax
from jax.experimental import pallas as pl
from jax.experimental.pallas import tpu as pltpu

S = 2048
M = 640
H = 32
D = 128
DC = 512
F = 1728
G = 2
NG = H // G
R = 128
TC = 256
EPS = 1e-5
NEG = -1e9
QSCALE = float(D ** -0.5 * math.log2(math.e))

f32 = jnp.float32
bf16 = jnp.bfloat16
_NT = (((1,), (1,)), ((), ()))


def _dot(a, b):
    return jnp.dot(a, b, preferred_element_type=f32)


def _recip(x):
    r = pltpu.reciprocal(x, approx=True)
    r = r * (2.0 - x * r)
    return r * (2.0 - x * r)


def _layernorm(x):
    mu = jnp.mean(x, axis=-1, keepdims=True)
    xc = x - mu
    var = jnp.mean(xc * xc, axis=-1, keepdims=True)
    return xc * lax.rsqrt(var + EPS)


def _gelu(x):
    c = math.sqrt(2.0 / math.pi)
    return 0.5 * x * (1.0 + jnp.tanh(c * (x + 0.044715 * (x * x * x))))


def _relayout(w_raw, half, kdim, pair, dst_ref):
    w = w_raw.at[half].reshape(kdim * 8, D)
    for p in range(G // 2):
        x = w[pl.ds(pair + p, kdim, stride=8), :]
        lo = pltpu.bitcast(x << 16, f32).astype(bf16)
        hi = pltpu.bitcast(x & jnp.uint32(0xFFFF0000), f32).astype(bf16)
        dst_ref[:, (2 * p) * D:(2 * p + 1) * D] = lo
        dst_ref[:, (2 * p + 1) * D:(2 * p + 2) * D] = hi


def _attention_group(g, q_s, k_s, v_s, ctx_s):
    nstrip = S // R
    items = [(u, i) for u in range(G) for i in range(nstrip - 1, -1, -1)]
    n = len(items)
    LA = 2
    st = {}
    row = lax.broadcasted_iota(jnp.int32, (R, R), 0)
    col = lax.broadcasted_iota(jnp.int32, (R, R), 1)
    causal = col <= row

    def scores(t):
        u, i = items[t]
        e = (i + 1) * R
        q = q_s[i * R:(i + 1) * R, u * D:(u + 1) * D]
        s = lax.dot_general(q, k_s[0:e, u * D:(u + 1) * D], _NT, preferred_element_type=f32)
        tiles = [s[:, j * 128:(j + 1) * 128] for j in range(i)]
        tiles.append(jnp.where(causal, s[:, e - R:e], NEG))
        st[t] = {"tiles": tiles}

    def rowmax(t):
        d = st[t]
        m = d["tiles"][0]
        for x in d["tiles"][1:]:
            m = jnp.maximum(m, x)
        d["m"] = jnp.max(m, axis=1, keepdims=True)

    def pv(t):
        u, i = items[t]
        d = st[t]
        e = (i + 1) * R
        ps = [jnp.exp2(x - d["m"]) for x in d["tiles"]]
        l = ps[0]
        for x in ps[1:]:
            l = l + x
        d["l"] = l
        p = jnp.concatenate(ps, axis=1).astype(bf16)
        d["o"] = _dot(p, v_s[0:e, u * D:(u + 1) * D])

    def finish(t):
        u, i = items[t]
        d = st.pop(t)
        lrow = jnp.sum(d["l"], axis=1, keepdims=True)
        ctx_s[g, i * R:(i + 1) * R, u * D:(u + 1) * D] = (d["o"] * _recip(lrow)).astype(bf16)

    for t in range(-LA, n + 1):
        if 0 <= t + LA < n:
            scores(t + LA)
        if 0 <= t + LA - 1 < n:
            rowmax(t + LA - 1)
        if 0 <= t < n:
            pv(t)
        if 0 <= t - 1 < n:
            finish(t - 1)


def _tail(x_s, ctx_s, wo_s, w1_s, w2_s, w3_s, w4_s, c_s, wmod_s, h1_s, out_s, o_hbm, osem):
    n = S // TC
    st = {}
    mod = _modulation(c_s, wmod_s[...])
    ga = mod[:, 0:M]
    sb = mod[:, M:2 * M]
    cb1 = 1.0 + mod[:, 2 * M:3 * M]
    gb = mod[:, 3 * M:4 * M]
    lane = lax.broadcasted_iota(jnp.int32, (1, 128), 1)
    out_copies = []

    def rows(t):
        return slice(t * TC, (t + 1) * TC)

    def oproj(t):
        acc = _dot(ctx_s[0, rows(t), :], wo_s[0:G * D, :])
        for g in range(1, NG):
            acc = acc + _dot(ctx_s[g, rows(t), :], wo_s[g * G * D:(g + 1) * G * D, :])
        x1 = x_s[rows(t), :].astype(f32) + ga * acc
        h = _layernorm(x1) * cb1 + sb
        st[t] = {"x1": x1, "h": h, "n1": _layernorm(h).astype(bf16)}

    def mm1(t):
        d = st[t]
        h1_s[8 + t * TC:8 + (t + 1) * TC, :] = _gelu(_dot(d.pop("n1"), w1_s[...]))

    def mm2(t):
        d = st[t]
        r0 = 8 + t * TC

        def ld(shift, tile):
            return h1_s[r0 + shift:r0 + shift + TC, tile * 128:(tile + 1) * 128]

        c = M // 4
        g = jnp.concatenate([
            ld(-1, 0),
            jnp.where(lane < c - 128, ld(-1, 1), ld(1, 1)),
            jnp.where(lane < 2 * c - 256, ld(1, 2), ld(-2, 2)),
            jnp.where(lane < 3 * c - 384, ld(-2, 3), ld(2, 3)),
            ld(2, 4),
        ], axis=1).astype(bf16)
        u = d.pop("h") + _dot(g, w2_s[...])
        d["u"] = u
        d["n2"] = _layernorm(u).astype(bf16)

    def mm3(t):
        d = st[t]
        a = lax.dot_general(d.pop("n2"), w3_s[...], _NT, preferred_element_type=f32)
        d["a"] = _gelu(a).astype(bf16)

    def mm4(t):
        d = st.pop(t)
        y = d["u"] + _dot(d["a"], w4_s[...])
        out_s[rows(t), :] = (d["x1"] + gb * y).astype(out_s.dtype)
        cp = pltpu.make_async_copy(out_s.at[rows(t), :], o_hbm.at[rows(t), :], osem.at[t])
        cp.start()
        out_copies.append(cp)

    for t in range(-2, n + 1):
        if 0 <= t + 2 < n:
            oproj(t + 2)
        if 0 <= t - 1 < n:
            mm3(t - 1)
        if 0 <= t + 1 < n:
            mm1(t + 1)
        if 0 <= t - 1 < n:
            mm4(t - 1)
        if 0 <= t < n:
            mm2(t)
    for cp in out_copies:
        cp.wait()


def _modulation(c_s, wmod):
    cv = c_s[...].astype(f32)
    sc = (cv * jax.nn.sigmoid(cv)).astype(bf16)
    return _dot(jnp.broadcast_to(sc, (16, M)), wmod)[0:1]


def _kernel(x_hbm, ckv_hbm, wq_hbm, wk_hbm, wv_hbm, wo_hbm, w1_hbm, w2_hbm, w3_hbm, w4_hbm, c_hbm, wmod_hbm,
            o_hbm,
            x_s, ckv_s, wq_raw, wk_raw, wv_raw, wo_s, w1_s, w2_s, w3_s, w4_s, c_s, wmod_a, wmod_b,
            h_s, wq_s, wk_s, wv_s, q_s, k_s, v_s, ctx_s, h1_s, out_s, sems, osem):
    h_s, wq_s, wk_s, wv_s, q_s, k_s, v_s, ctx_s = (r.bitcast(bf16) for r in (h_s, wq_s, wk_s, wv_s, q_s, k_s, v_s, ctx_s))
    wq32, wk32, wv32 = (w.bitcast(jnp.uint32) for w in (wq_hbm, wk_hbm, wv_hbm))
    hp = H // 4
    moves = [
        (ckv_hbm, ckv_s),
        (wk32.at[:, 0:hp, :], wk_raw.at[0]),
        (wv32.at[:, 0:hp, :], wv_raw.at[0]),
        (x_hbm, x_s),
        (c_hbm, c_s),
        (wmod_hbm.at[:, 0:2 * M], wmod_a),
        (wq32.at[:, 0:hp, :], wq_raw.at[0]),
        (wk32.at[:, hp:2 * hp, :], wk_raw.at[1]),
        (wv32.at[:, hp:2 * hp, :], wv_raw.at[1]),
        (wq32.at[:, hp:2 * hp, :], wq_raw.at[1]),
        (wo_hbm, wo_s),
        (wmod_hbm.at[:, 2 * M:6 * M], wmod_b),
        (w1_hbm, w1_s),
        (w2_hbm, w2_s),
        (w3_hbm, w3_s),
        (w4_hbm, w4_s),
    ]
    copies = [pltpu.make_async_copy(src, dst, sems.at[i]) for i, (src, dst) in enumerate(moves)]
    for cp in copies[:7]:
        cp.start()
    (cp_ckv, cp_wk0, cp_wv0, cp_x, cp_c, cp_wma, cp_wq0, cp_wk1, cp_wv1, cp_wq1) = copies[:10]

    def k_proj(half, pair):
        _relayout(wk_raw, half, DC, pair, wk_s)
        k_s[...] = _dot(ckv_s[...], wk_s[...]).astype(bf16)

    def v_proj(half, pair):
        _relayout(wv_raw, half, DC, pair, wv_s)
        v_s[...] = _dot(ckv_s[...], wv_s[...]).astype(bf16)

    def q_proj(half, pair):
        _relayout(wq_raw, half, M, pair, wq_s)
        q_s[...] = (_dot(h_s[...], wq_s[...]) * QSCALE).astype(bf16)

    h1_s[0:8, :] = jnp.zeros((8, M), f32)
    h1_s[8 + S:16 + S, :] = jnp.zeros((8, M), f32)

    cp_ckv.wait()
    cp_wk0.wait()
    k_proj(0, 0)
    cp_wv0.wait()
    v_proj(0, 0)
    cp_x.wait()
    cp_c.wait()
    cp_wma.wait()
    mod = _modulation(c_s, wmod_a[...])
    sa = mod[:, 0:M]
    ca1 = 1.0 + mod[:, M:2 * M]
    LC = 256

    def ln_chunk(i):
        xi = x_s[i * LC:(i + 1) * LC, :].astype(f32)
        h_s[i * LC:(i + 1) * LC, :] = (_layernorm(xi) * ca1 + sa).astype(bf16)

    ln_chunk(0)
    ln_chunk(1)
    cp_wq0.wait()
    _relayout(wq_raw, 0, M, 0, wq_s)
    for i in range(S // LC):
        if i + 2 < S // LC:
            ln_chunk(i + 2)
        rs = slice(i * LC, (i + 1) * LC)
        q_s[rs, :] = (_dot(h_s[rs, :], wq_s[...]) * QSCALE).astype(bf16)

    def group(g, carry):
        @pl.when(g == 0)
        def _():
            for cp in copies[7:10]:
                cp.start()

        @pl.when(g == 1)
        def _():
            for cp in copies[7:10]:
                cp.wait()
            for cp in copies[10:]:
                cp.start()

        _attention_group(g, q_s, k_s, v_s, ctx_s)
        half = (g + 1) // (NG // 2)
        pair = ((g + 1) % (NG // 2)) * (G // 2)
        k_proj(half, pair)
        q_proj(half, pair)
        v_proj(half, pair)
        return carry

    lax.fori_loop(0, NG - 1, group, 0)
    _attention_group(NG - 1, q_s, k_s, v_s, ctx_s)

    for cp in copies[10:]:
        cp.wait()
    _tail(x_s, ctx_s, wo_s, w1_s, w2_s, w3_s, w4_s, c_s, wmod_b, h1_s, out_s, o_hbm, osem)


@jax.jit
def pallas_adaLN_cond__compressed_kv_cla__mixer_s_mlp__prompt_kernel(
    A_x: jax.Array,
    A_c_kv: jax.Array,
    A_w_q: jax.Array,
    A_w_uk: jax.Array,
    A_w_uv: jax.Array,
    A_w_o: jax.Array,
    B_x: jax.Array,
    B_w1: jax.Array,
    B_w2: jax.Array,
    B_w3: jax.Array,
    B_w4: jax.Array,
    c: jax.Array,
    w_mod: jax.Array,
):
    del B_x
    x = A_x.reshape(S, M)
    ckv = A_c_kv.reshape(S, DC)
    wo = A_w_o.reshape(H * D, M)

    any_spec = pl.BlockSpec(memory_space=pl.ANY)
    scratch = [
        pltpu.VMEM((S, M), bf16),
        pltpu.VMEM((S, DC), bf16),
        pltpu.VMEM((2, M, 8, D), jnp.uint32),
        pltpu.VMEM((2, DC, 8, D), jnp.uint32),
        pltpu.VMEM((2, DC, 8, D), jnp.uint32),
        pltpu.VMEM((H * D, M), bf16),
        pltpu.VMEM((M, M), bf16),
        pltpu.VMEM((M, M), bf16),
        pltpu.VMEM((F, M), bf16),
        pltpu.VMEM((F, M), bf16),
        pltpu.VMEM((1, M), bf16),
        pltpu.VMEM((M, 2 * M), bf16),
        pltpu.VMEM((M, 4 * M), bf16),
        pltpu.VMEM((S // 2, M), jnp.uint32),
        pltpu.VMEM((M // 2, G * D), jnp.uint32),
        pltpu.VMEM((DC // 2, G * D), jnp.uint32),
        pltpu.VMEM((DC // 2, G * D), jnp.uint32),
        pltpu.VMEM((S // 2, G * D), jnp.uint32),
        pltpu.VMEM((S // 2, G * D), jnp.uint32),
        pltpu.VMEM((S // 2, G * D), jnp.uint32),
        pltpu.VMEM((NG, S // 2, G * D), jnp.uint32),
        pltpu.VMEM((S + 16, M), f32),
        pltpu.VMEM((S, M), bf16),
        pltpu.SemaphoreType.DMA((16,)),
        pltpu.SemaphoreType.DMA((S // TC,)),
    ]
    out = pl.pallas_call(
        _kernel,
        out_shape=jax.ShapeDtypeStruct((S, M), A_x.dtype),
        in_specs=[any_spec] * 12,
        out_specs=any_spec,
        scratch_shapes=scratch,
        compiler_params=pltpu.CompilerParams(vmem_limit_bytes=126 * 1024 * 1024),
    )(x, ckv, A_w_q, A_w_uk, A_w_uv, wo, B_w1, B_w2, B_w3.T, B_w4, c, w_mod)
    return out.reshape(1, S, M)
```

```python
import functools
import math

import jax
import jax.numpy as jnp
import numpy as np
from jax import lax
from jax.experimental import pallas as pl
from jax.experimental.pallas import tpu as pltpu

S = 2048
M = 640
H = 32
D = 128
DC = 512
F = 1728
G = 2
NG = H // G
R = 128
TC = 256
TIE = 6
NPRE = 4
PEND = 2
EPS = 1e-5
NEG = -1e9
QSCALE = float(D ** -0.5 * math.log2(math.e))

f32 = jnp.float32
bf16 = jnp.bfloat16
_NT = (((1,), (1,)), ((), ()))


def _dot(a, b):
    return jnp.dot(a, b, preferred_element_type=f32)


def _recip(x):
    r = pltpu.reciprocal(x, approx=True)
    r = r * (2.0 - x * r)
    return r * (2.0 - x * r)


def _layernorm(x):
    mu = jnp.mean(x, axis=-1, keepdims=True)
    xc = x - mu
    var = jnp.mean(xc * xc, axis=-1, keepdims=True)
    return xc * lax.rsqrt(var + EPS)


def _gelu(x):
    c = math.sqrt(2.0 / math.pi)
    return 0.5 * x * (1.0 + jnp.tanh(c * (x + 0.044715 * (x * x * x))))


def _relayout(w_raw, half, kdim, pair, dst_ref):
    w = w_raw.at[half].reshape(kdim * 8, D)
    for p in range(G // 2):
        x = w[pl.ds(pair + p, kdim, stride=8), :]
        lo = pltpu.bitcast(x << 16, f32).astype(bf16)
        hi = pltpu.bitcast(x & jnp.uint32(0xFFFF0000), f32).astype(bf16)
        dst_ref[:, (2 * p) * D:(2 * p + 1) * D] = lo
        dst_ref[:, (2 * p + 1) * D:(2 * p + 2) * D] = hi


def _attention_group(g, q_s, k_s, v_s, ctx_s):
    nstrip = S // R
    items = [(u, i) for u in range(G) for i in range(nstrip - 1, -1, -1)]
    n = len(items)
    LA = 2
    st = {}
    inv = {}
    row = lax.broadcasted_iota(jnp.int32, (R, R), 0)
    col = lax.broadcasted_iota(jnp.int32, (R, R), 1)
    causal = col <= row

    def scores(t):
        u, i = items[t]
        e = (i + 1) * R
        q = q_s[i * R:(i + 1) * R, u * D:(u + 1) * D]
        s = lax.dot_general(q, k_s[0:e, u * D:(u + 1) * D], _NT, preferred_element_type=f32)
        tiles = [s[:, j * 128:(j + 1) * 128] for j in range(i)]
        tiles.append(jnp.where(causal, s[:, e - R:e], NEG))
        st[t] = {"tiles": tiles}

    def rowmax(t):
        d = st[t]
        m = d["tiles"][0]
        for x in d["tiles"][1:]:
            m = jnp.maximum(m, x)
        mm = jnp.max(m, axis=1, keepdims=True)
        if (t - TIE) in inv:
            mm = mm + 0.0 * inv.pop(t - TIE)
        d["m"] = mm

    def pv(t):
        u, i = items[t]
        d = st[t]
        e = (i + 1) * R
        ps = [jnp.exp2(x - d["m"]) for x in d["tiles"]]
        l = ps[0]
        for x in ps[1:]:
            l = l + x
        d["inv"] = _recip(jnp.sum(l, axis=1, keepdims=True))
        inv[t] = d["inv"]
        p = jnp.concatenate(ps, axis=1).astype(bf16)
        d["o"] = _dot(p, v_s[0:e, u * D:(u + 1) * D])

    def finish(t):
        u, i = items[t]
        d = st.pop(t)
        ctx_s[g, i * R:(i + 1) * R, u * D:(u + 1) * D] = (d["o"] * d["inv"]).astype(bf16)

    for t in range(-LA, n + 1):
        if 0 <= t + LA < n:
            scores(t + LA)
        if 0 <= t + LA - 1 < n:
            rowmax(t + LA - 1)
        if 0 <= t < n:
            pv(t)
        if 0 <= t - 1 < n:
            finish(t - 1)


def _tail(x_s, ctx_s, wo_s, w1_s, w2_s, w3_s, w4_s, c_s, wmod_s, h1_s, out_s, o_hbm, osem):
    n = S // TC
    PR = 16
    st = {}
    mod = _modulation(c_s, wmod_s[...])
    ga = mod[:, 0:M]
    sb = mod[:, M:2 * M]
    cb1 = 1.0 + mod[:, 2 * M:3 * M]
    gb = mod[:, 3 * M:4 * M]
    lane = lax.broadcasted_iota(jnp.int32, (1, 128), 1)
    out_copies = []
    pending = []

    def run_pending(k):
        for _ in range(min(k, len(pending))):
            pending.pop(0)()

    def rows(t):
        return slice(t * TC, (t + 1) * TC)

    def oproj(t):
        acc = None
        for g in range(NG):
            part = _dot(ctx_s[g, rows(t), :], wo_s[g * G * D:(g + 1) * G * D, :])
            acc = part if acc is None else acc + part
            run_pending(PEND)
        d = st[t] = {"x1": [], "h": [], "n1": []}

        def piece(j):
            r = slice(j * PR, (j + 1) * PR)
            x1 = x_s[t * TC + j * PR:t * TC + (j + 1) * PR, :].astype(f32) + ga * acc[r]
            h = _layernorm(x1) * cb1 + sb
            d["x1"].append(x1)
            d["h"].append(h)
            d["n1"].append(_layernorm(h).astype(bf16))

        pending.extend(functools.partial(piece, j) for j in range(TC // PR))

    def mm1(t):
        run_pending(len(pending))
        d = st[t]
        h1_s[8 + t * TC:8 + (t + 1) * TC, :] = _gelu(_dot(jnp.concatenate(d.pop("n1"), axis=0), w1_s[...]))

    def mm2(t):
        d = st[t]
        r0 = 8 + t * TC

        def ld(shift, tile):
            return h1_s[r0 + shift:r0 + shift + TC, tile * 128:(tile + 1) * 128]

        c = M // 4
        g = jnp.concatenate([
            ld(-1, 0),
            jnp.where(lane < c - 128, ld(-1, 1), ld(1, 1)),
            jnp.where(lane < 2 * c - 256, ld(1, 2), ld(-2, 2)),
            jnp.where(lane < 3 * c - 384, ld(-2, 3), ld(2, 3)),
            ld(2, 4),
        ], axis=1).astype(bf16)
        hs = _dot(g, w2_s[...])
        d["u"] = []
        d["n2"] = []

        def piece(j):
            u = d["h"][j] + hs[j * PR:(j + 1) * PR]
            d["u"].append(u)
            d["n2"].append(_layernorm(u).astype(bf16))

        pending.extend(functools.partial(piece, j) for j in range(TC // PR))

    def mm3(t):
        d = st[t]
        while len(d["n2"]) < TC // PR:
            run_pending(1)
        a = lax.dot_general(jnp.concatenate(d.pop("n2"), axis=0), w3_s[...], _NT, preferred_element_type=f32)
        d["a"] = _gelu(a).astype(bf16)

    def mm4(t):
        d = st.pop(t)
        y = jnp.concatenate(d["u"], axis=0) + _dot(d["a"], w4_s[...])
        out_s[rows(t), :] = (jnp.concatenate(d["x1"], axis=0) + gb * y).astype(out_s.dtype)
        cp = pltpu.make_async_copy(out_s.at[rows(t), :], o_hbm.at[rows(t), :], osem.at[t])
        cp.start()
        out_copies.append(cp)

    for t in range(-2, n + 1):
        if 0 <= t + 2 < n:
            oproj(t + 2)
        if 0 <= t - 1 < n:
            mm3(t - 1)
        if 0 <= t + 1 < n:
            mm1(t + 1)
        if 0 <= t - 1 < n:
            mm4(t - 1)
        if 0 <= t < n:
            mm2(t)
    for cp in out_copies:
        cp.wait()


def _modulation(c_s, wmod):
    cv = c_s[...].astype(f32)
    sc = (cv * jax.nn.sigmoid(cv)).astype(bf16)
    return _dot(jnp.broadcast_to(sc, (16, M)), wmod)[0:1]


def _kernel(x_hbm, ckv_hbm, wq_hbm, wk_hbm, wv_hbm, wo_hbm, w1_hbm, w2_hbm, w3_hbm, w4_hbm, c_hbm, wmod_hbm,
            o_hbm,
            x_s, ckv_s, wq_raw, wk_raw, wv_raw, wo_s, w1_s, w2_s, w3_s, w4_s, c_s, wmod_a, wmod_b,
            h_s, wq_s, wk_s, wv_s, q_s, k_s, v_s, ctx_s, h1_s, out_s, sems, osem):
    h_s, wq_s, wk_s, wv_s, q_s, k_s, v_s, ctx_s = (r.bitcast(bf16) for r in (h_s, wq_s, wk_s, wv_s, q_s, k_s, v_s, ctx_s))
    u32 = jnp.uint32
    wq32, wk32, wv32 = (w.bitcast(u32) for w in (wq_hbm, wk_hbm, wv_hbm))
    first = [
        (x_hbm, x_s),
        (c_hbm, c_s),
        (wmod_hbm.at[:, 0:2 * M], wmod_a),
        (wq32.at[:, 0:4, :], wq_raw.at[0, :, 0:4, :]),
        (ckv_hbm.bitcast(u32), ckv_s),
        (wk32.at[:, 0:4, :], wk_raw.at[0, :, 0:4, :]),
        (wv32.at[:, 0:4, :], wv_raw.at[0, :, 0:4, :]),
    ]
    later = [
        (wk32.at[:, 4:8, :], wk_raw.at[0, :, 4:8, :]),
        (wq32.at[:, 4:8, :], wq_raw.at[0, :, 4:8, :]),
        (wv32.at[:, 4:8, :], wv_raw.at[0, :, 4:8, :]),
        (wk32.at[:, 8:16, :], wk_raw.at[1]),
        (wq32.at[:, 8:16, :], wq_raw.at[1]),
        (wv32.at[:, 8:16, :], wv_raw.at[1]),
    ]
    last = [
        (wo_hbm.bitcast(u32), wo_s),
        (wmod_hbm.at[:, 2 * M:6 * M], wmod_b),
        (w1_hbm.bitcast(u32), w1_s),
        (w2_hbm.bitcast(u32), w2_s),
        (w3_hbm.bitcast(u32), w3_s),
        (w4_hbm.bitcast(u32), w4_s),
    ]
    copies = [pltpu.make_async_copy(src, dst, sems.at[i]) for i, (src, dst) in enumerate(first + later + last)]
    for cp in copies:
        cp.start()
    cp_x, cp_c, cp_wma, cp_ckv, cp_wk0, cp_wv0 = (copies[i] for i in (0, 1, 2, 4, 5, 6))
    cp_wq0 = copies[3]
    cp_later = copies[len(first):len(first) + len(later)]
    cp_last = copies[len(first) + len(later):]
    ckv_s, wo_s, w1_s, w2_s, w3_s, w4_s, h_s, wq_s, wk_s, wv_s, q_s, k_s, v_s, ctx_s = (
        r.bitcast(bf16) for r in (ckv_s, wo_s, w1_s, w2_s, w3_s, w4_s, h_s, wq_s, wk_s, wv_s, q_s, k_s, v_s, ctx_s))

    def k_proj(half, pair):
        _relayout(wk_raw, half, DC, pair, wk_s)
        k_s[...] = _dot(ckv_s[...], wk_s[...]).astype(bf16)

    def v_proj(half, pair):
        _relayout(wv_raw, half, DC, pair, wv_s)
        v_s[...] = _dot(ckv_s[...], wv_s[...]).astype(bf16)

    def q_proj(half, pair):
        _relayout(wq_raw, half, M, pair, wq_s)
        q_s[...] = (_dot(h_s[...], wq_s[...]) * QSCALE).astype(bf16)

    h1_s[0:8, :] = jnp.zeros((8, M), f32)
    h1_s[8 + S:16 + S, :] = jnp.zeros((8, M), f32)

    cp_x.wait()
    cp_c.wait()
    cp_wma.wait()
    mod = _modulation(c_s, wmod_a[...])
    sa = mod[:, 0:M]
    ca1 = 1.0 + mod[:, M:2 * M]
    LC = 256

    def ln_chunk(i):
        xi = x_s[i * LC:(i + 1) * LC, :].astype(f32)
        h_s[i * LC:(i + 1) * LC, :] = (_layernorm(xi) * ca1 + sa).astype(bf16)

    for i in range(NPRE):
        ln_chunk(i)
    cp_wq0.wait()
    _relayout(wq_raw, 0, M, 0, wq_s)
    for i in range(S // LC):
        if i + NPRE < S // LC:
            ln_chunk(i + NPRE)
        rs = slice(i * LC, (i + 1) * LC)
        q_s[rs, :] = (_dot(h_s[rs, :], wq_s[...]) * QSCALE).astype(bf16)
    cp_ckv.wait()
    cp_wk0.wait()
    k_proj(0, 0)
    cp_wv0.wait()
    v_proj(0, 0)

    def group(g, carry):
        @pl.when(g == 2)
        def _():
            for cp in cp_later:
                cp.wait()

        @pl.when(g == 8)
        def _():
            for cp in cp_last:
                cp.wait()

        _attention_group(g, q_s, k_s, v_s, ctx_s)
        half = (g + 1) // (NG // 2)
        pair = ((g + 1) % (NG // 2)) * (G // 2)
        k_proj(half, pair)
        q_proj(half, pair)
        v_proj(half, pair)
        return carry

    lax.fori_loop(0, NG - 1, group, 0)
    _attention_group(NG - 1, q_s, k_s, v_s, ctx_s)

    _tail(x_s, ctx_s, wo_s, w1_s, w2_s, w3_s, w4_s, c_s, wmod_b, h1_s, out_s, o_hbm, osem)


@jax.jit
def pallas_adaLN_cond__compressed_kv_cla__mixer_s_mlp__prompt_kernel(
    A_x: jax.Array,
    A_c_kv: jax.Array,
    A_w_q: jax.Array,
    A_w_uk: jax.Array,
    A_w_uv: jax.Array,
    A_w_o: jax.Array,
    B_x: jax.Array,
    B_w1: jax.Array,
    B_w2: jax.Array,
    B_w3: jax.Array,
    B_w4: jax.Array,
    c: jax.Array,
    w_mod: jax.Array,
):
    del B_x
    x = A_x.reshape(S, M)
    ckv = A_c_kv.reshape(S, DC)
    wo = A_w_o.reshape(H * D, M)

    any_spec = pl.BlockSpec(memory_space=pl.ANY)
    scratch = [
        pltpu.VMEM((S, M), bf16),
        pltpu.VMEM((S // 2, DC), jnp.uint32),
        pltpu.VMEM((2, M, 8, D), jnp.uint32),
        pltpu.VMEM((2, DC, 8, D), jnp.uint32),
        pltpu.VMEM((2, DC, 8, D), jnp.uint32),
        pltpu.VMEM((H * D // 2, M), jnp.uint32),
        pltpu.VMEM((M // 2, M), jnp.uint32),
        pltpu.VMEM((M // 2, M), jnp.uint32),
        pltpu.VMEM((F // 2, M), jnp.uint32),
        pltpu.VMEM((F // 2, M), jnp.uint32),
        pltpu.VMEM((1, M), bf16),
        pltpu.VMEM((M, 2 * M), bf16),
        pltpu.VMEM((M, 4 * M), bf16),
        pltpu.VMEM((S // 2, M), jnp.uint32),
        pltpu.VMEM((M // 2, G * D), jnp.uint32),
        pltpu.VMEM((DC // 2, G * D), jnp.uint32),
        pltpu.VMEM((DC // 2, G * D), jnp.uint32),
        pltpu.VMEM((S // 2, G * D), jnp.uint32),
        pltpu.VMEM((S // 2, G * D), jnp.uint32),
        pltpu.VMEM((S // 2, G * D), jnp.uint32),
        pltpu.VMEM((NG, S // 2, G * D), jnp.uint32),
        pltpu.VMEM((S + 16, M), f32),
        pltpu.VMEM((S, M), bf16),
        pltpu.SemaphoreType.DMA((19,)),
        pltpu.SemaphoreType.DMA((S // TC,)),
    ]
    out = pl.pallas_call(
        _kernel,
        out_shape=jax.ShapeDtypeStruct((S, M), A_x.dtype),
        in_specs=[any_spec] * 12,
        out_specs=any_spec,
        scratch_shapes=scratch,
        compiler_params=pltpu.CompilerParams(vmem_limit_bytes=126 * 1024 * 1024),
    )(x, ckv, A_w_q, A_w_uk, A_w_uv, wo, B_w1, B_w2, B_w3.T, B_w4, c, w_mod)
    return out.reshape(1, S, M)
```

```python
import functools
import math

import jax
import jax.numpy as jnp
import numpy as np
from jax import lax
from jax.experimental import pallas as pl
from jax.experimental.pallas import tpu as pltpu

S = 2048
M = 640
H = 32
D = 128
DC = 512
F = 1728
G = 2
NG = H // G
R = 128
TC = 256
TIE = 6
LA = 1
ORDER = 0
LC = 128
KC = 1024
NX = 4
PEND = 2
EPS = 1e-5
NEG = -1e9
QSCALE = float(D ** -0.5 * math.log2(math.e))

f32 = jnp.float32
bf16 = jnp.bfloat16
_NT = (((1,), (1,)), ((), ()))


def _dot(a, b):
    return jnp.dot(a, b, preferred_element_type=f32)


def _recip(x):
    r = pltpu.reciprocal(x, approx=True)
    r = r * (2.0 - x * r)
    return r * (2.0 - x * r)


def _layernorm(x):
    mu = jnp.mean(x, axis=-1, keepdims=True)
    xc = x - mu
    var = jnp.mean(xc * xc, axis=-1, keepdims=True)
    return xc * lax.rsqrt(var + EPS)


def _gelu(x):
    c = math.sqrt(2.0 / math.pi)
    return 0.5 * x * (1.0 + jnp.tanh(c * (x + 0.044715 * (x * x * x))))


def _relayout(w_raw, half, kdim, pair, dst_ref):
    w = w_raw.at[half].reshape(kdim * 8, D)
    for p in range(G // 2):
        x = w[pl.ds(pair + p, kdim, stride=8), :]
        lo = pltpu.bitcast(x << 16, f32).astype(bf16)
        hi = pltpu.bitcast(x & jnp.uint32(0xFFFF0000), f32).astype(bf16)
        dst_ref[:, (2 * p) * D:(2 * p + 1) * D] = lo
        dst_ref[:, (2 * p + 1) * D:(2 * p + 2) * D] = hi


def _attention_group(g, q_s, k_s, v_s, ctx_s, fillers=()):
    nstrip = S // R
    desc, asc = range(nstrip - 1, -1, -1), range(nstrip)
    orders = [(desc, desc), (asc, desc), (desc, asc), (asc, asc)][ORDER]
    items = [(u, i) for u in range(G) for i in orders[u]]
    n = len(items)
    st = {}
    inv = {}
    row = lax.broadcasted_iota(jnp.int32, (R, R), 0)
    col = lax.broadcasted_iota(jnp.int32, (R, R), 1)
    causal = col <= row

    def scores(t):
        u, i = items[t]
        e = (i + 1) * R
        q = q_s[i * R:(i + 1) * R, u * D:(u + 1) * D]
        s = lax.dot_general(q, k_s[0:e, u * D:(u + 1) * D], _NT, preferred_element_type=f32)
        tiles = [s[:, j * 128:(j + 1) * 128] for j in range(i)]
        tiles.append(jnp.where(causal, s[:, e - R:e], NEG))
        st[t] = {"tiles": tiles}

    def rowmax(t):
        d = st[t]
        m = d["tiles"][0]
        for x in d["tiles"][1:]:
            m = jnp.maximum(m, x)
        mm = jnp.max(m, axis=1, keepdims=True)
        if (t - TIE) in inv:
            mm = mm + 0.0 * inv.pop(t - TIE)
        d["m"] = mm

    def pv(t):
        u, i = items[t]
        d = st[t]
        e = (i + 1) * R
        ps = [jnp.exp2(x - d["m"]) for x in d["tiles"]]
        l = ps[0]
        for x in ps[1:]:
            l = l + x
        d["inv"] = _recip(jnp.sum(l, axis=1, keepdims=True))
        inv[t] = d["inv"]
        p = jnp.concatenate(ps, axis=1).astype(bf16)
        d["o"] = _dot(p, v_s[0:e, u * D:(u + 1) * D])

    def finish(t):
        u, i = items[t]
        d = st.pop(t)
        ctx_s[g, i * R:(i + 1) * R, u * D:(u + 1) * D] = (d["o"] * d["inv"]).astype(bf16)

    fillers = list(fillers)
    for t in range(-LA, n + 1):
        if 0 <= t + LA < n:
            scores(t + LA)
        if t + LA >= n - 1 and fillers:
            fillers.pop(0)()
        if 0 <= t + LA - 1 < n:
            rowmax(t + LA - 1)
        if 0 <= t < n:
            pv(t)
        if 0 <= t - 1 < n:
            finish(t - 1)
    for f in fillers:
        f()


def _tail(x_s, ctx_s, wo_s, w1_s, w2_s, w3_s, w4_s, c_s, wmod_s, h1_s, out_s, o_hbm, osem):
    n = S // TC
    PR = 16
    st = {}
    mod = _modulation(c_s, wmod_s[...])
    ga = mod[:, 0:M]
    sb = mod[:, M:2 * M]
    cb1 = 1.0 + mod[:, 2 * M:3 * M]
    gb = mod[:, 3 * M:4 * M]
    lane = lax.broadcasted_iota(jnp.int32, (1, 128), 1)
    out_copies = []
    pending = []

    def run_pending(k):
        for _ in range(min(k, len(pending))):
            pending.pop(0)()

    def rows(t):
        return slice(t * TC, (t + 1) * TC)

    def oproj(t):
        acc = None
        for g in range(NG):
            part = _dot(ctx_s[g, rows(t), :], wo_s[g * G * D:(g + 1) * G * D, :])
            acc = part if acc is None else acc + part
            run_pending(PEND)
        d = st[t] = {"x1": [], "h": [], "n1": []}

        def piece(j):
            r = slice(j * PR, (j + 1) * PR)
            x1 = x_s[t * TC + j * PR:t * TC + (j + 1) * PR, :].astype(f32) + ga * acc[r]
            h = _layernorm(x1) * cb1 + sb
            d["x1"].append(x1)
            d["h"].append(h)
            d["n1"].append(_layernorm(h).astype(bf16))

        pending.extend(functools.partial(piece, j) for j in range(TC // PR))

    def mm1(t):
        run_pending(len(pending))
        d = st[t]
        h1_s[8 + t * TC:8 + (t + 1) * TC, :] = _gelu(_dot(jnp.concatenate(d.pop("n1"), axis=0), w1_s[...]))

    def mm2(t):
        d = st[t]
        r0 = 8 + t * TC

        def ld(shift, tile):
            return h1_s[r0 + shift:r0 + shift + TC, tile * 128:(tile + 1) * 128]

        c = M // 4
        g = jnp.concatenate([
            ld(-1, 0),
            jnp.where(lane < c - 128, ld(-1, 1), ld(1, 1)),
            jnp.where(lane < 2 * c - 256, ld(1, 2), ld(-2, 2)),
            jnp.where(lane < 3 * c - 384, ld(-2, 3), ld(2, 3)),
            ld(2, 4),
        ], axis=1).astype(bf16)
        hs = _dot(g, w2_s[...])
        d["u"] = []
        d["n2"] = []

        def piece(j):
            u = d["h"][j] + hs[j * PR:(j + 1) * PR]
            d["u"].append(u)
            d["n2"].append(_layernorm(u).astype(bf16))

        pending.extend(functools.partial(piece, j) for j in range(TC // PR))

    def mm3(t):
        d = st[t]
        while len(d["n2"]) < TC // PR:
            run_pending(1)
        a = lax.dot_general(jnp.concatenate(d.pop("n2"), axis=0), w3_s[...], _NT, preferred_element_type=f32)
        d["a"] = _gelu(a).astype(bf16)

    def mm4(t):
        d = st.pop(t)
        y = jnp.concatenate(d["u"], axis=0) + _dot(d["a"], w4_s[...])
        out_s[rows(t), :] = (jnp.concatenate(d["x1"], axis=0) + gb * y).astype(out_s.dtype)
        cp = pltpu.make_async_copy(out_s.at[rows(t), :], o_hbm.at[rows(t), :], osem.at[t])
        cp.start()
        out_copies.append(cp)

    for t in range(-2, n + 1):
        if 0 <= t + 2 < n:
            oproj(t + 2)
        if 0 <= t - 1 < n:
            mm3(t - 1)
        if 0 <= t + 1 < n:
            mm1(t + 1)
        if 0 <= t - 1 < n:
            mm4(t - 1)
        if 0 <= t < n:
            mm2(t)
    for cp in out_copies:
        cp.wait()


def _modulation(c_s, wmod):
    cv = c_s[...].astype(f32)
    sc = (cv * jax.nn.sigmoid(cv)).astype(bf16)
    return _dot(jnp.broadcast_to(sc, (16, M)), wmod)[0:1]


def _kernel(x_hbm, ckv_hbm, wq_hbm, wk_hbm, wv_hbm, wo_hbm, w1_hbm, w2_hbm, w3_hbm, w4_hbm, c_hbm, wmod_hbm,
            o_hbm,
            x_s, ckv_s, wq_raw, wk_raw, wv_raw, wo_s, w1_s, w2_s, w3_s, w4_s, c_s, wmod_a, wmod_b,
            h_s, wq_s, wk_s, wv_s, q_s, k_s, v_s, ctx_s, h1_s, out_s, sems, osem):
    h_s, wq_s, wk_s, wv_s, q_s, k_s, v_s, ctx_s = (r.bitcast(bf16) for r in (h_s, wq_s, wk_s, wv_s, q_s, k_s, v_s, ctx_s))
    u32 = jnp.uint32
    wq32, wk32, wv32 = (w.bitcast(u32) for w in (wq_hbm, wk_hbm, wv_hbm))
    XC = S // NX
    first = [
        (ckv_hbm.bitcast(u32), ckv_s),
        (wk32.at[:, 0:4, :], wk_raw.at[0, :, 0:4, :]),
        (wv32.at[:, 0:4, :], wv_raw.at[0, :, 0:4, :]),
        (c_hbm, c_s),
        (wmod_hbm.at[:, 0:2 * M], wmod_a),
        (wq32.at[:, 0:4, :], wq_raw.at[0, :, 0:4, :]),
    ] + [(x_hbm.at[j * XC:(j + 1) * XC, :], x_s.at[j * XC:(j + 1) * XC, :]) for j in range(NX)]
    later = [
        (wk32.at[:, 4:8, :], wk_raw.at[0, :, 4:8, :]),
        (wq32.at[:, 4:8, :], wq_raw.at[0, :, 4:8, :]),
        (wv32.at[:, 4:8, :], wv_raw.at[0, :, 4:8, :]),
        (wk32.at[:, 8:16, :], wk_raw.at[1]),
        (wq32.at[:, 8:16, :], wq_raw.at[1]),
        (wv32.at[:, 8:16, :], wv_raw.at[1]),
    ]
    last = [
        (wo_hbm.bitcast(u32), wo_s),
        (wmod_hbm.at[:, 2 * M:6 * M], wmod_b),
        (w1_hbm.bitcast(u32), w1_s),
        (w2_hbm.bitcast(u32), w2_s),
        (w3_hbm.bitcast(u32), w3_s),
        (w4_hbm.bitcast(u32), w4_s),
    ]
    copies = [pltpu.make_async_copy(src, dst, sems.at[i]) for i, (src, dst) in enumerate(first + later + last)]
    for cp in copies:
        cp.start()
    cp_ckv, cp_wk0, cp_wv0, cp_c, cp_wma, cp_wq0 = copies[:6]
    cp_x = copies[6:6 + NX]
    cp_later = copies[len(first):len(first) + len(later)]
    cp_last = copies[len(first) + len(later):]
    ckv_s, wo_s, w1_s, w2_s, w3_s, w4_s, h_s, wq_s, wk_s, wv_s, q_s, k_s, v_s, ctx_s = (
        r.bitcast(bf16) for r in (ckv_s, wo_s, w1_s, w2_s, w3_s, w4_s, h_s, wq_s, wk_s, wv_s, q_s, k_s, v_s, ctx_s))

    def k_proj(half, pair):
        _relayout(wk_raw, half, DC, pair, wk_s)
        k_s[...] = _dot(ckv_s[...], wk_s[...]).astype(bf16)

    def v_proj(half, pair):
        _relayout(wv_raw, half, DC, pair, wv_s)
        v_s[...] = _dot(ckv_s[...], wv_s[...]).astype(bf16)

    def q_proj(half, pair):
        _relayout(wq_raw, half, M, pair, wq_s)
        q_s[...] = (_dot(h_s[...], wq_s[...]) * QSCALE).astype(bf16)

    h1_s[0:8, :] = jnp.zeros((8, M), f32)
    h1_s[8 + S:16 + S, :] = jnp.zeros((8, M), f32)

    cp_ckv.wait()
    cp_wk0.wait()
    k_proj(0, 0)
    cp_wv0.wait()
    v_proj(0, 0)
    cp_c.wait()
    cp_wma.wait()
    cp_wq0.wait()
    mod = _modulation(c_s, wmod_a[...])
    sa = mod[:, 0:M]
    ca1 = 1.0 + mod[:, M:2 * M]
    _relayout(wq_raw, 0, M, 0, wq_s)
    def ln_rows(r0):
        xi = x_s[r0:r0 + LC, :].astype(f32)
        h_s[r0:r0 + LC, :] = (_layernorm(xi) * ca1 + sa).astype(bf16)

    for j in range(NX):
        cp_x[j].wait()
        starts = list(range(j * XC, (j + 1) * XC, LC))
        ln_rows(starts[0])
        for i, r0 in enumerate(starts):
            if i + 1 < len(starts):
                ln_rows(starts[i + 1])
            q_s[r0:r0 + LC, :] = (_dot(h_s[r0:r0 + LC, :], wq_s[...]) * QSCALE).astype(bf16)

    def group(g, carry):
        @pl.when(g == 2)
        def _():
            for cp in cp_later:
                cp.wait()

        @pl.when(g == 8)
        def _():
            for cp in cp_last:
                cp.wait()

        half = (g + 1) // (NG // 2)
        pair = ((g + 1) % (NG // 2)) * (G // 2)
        _relayout(wk_raw, half, DC, pair, wk_s)

        def k_rows(r0):
            k_s[r0:r0 + KC, :] = _dot(ckv_s[r0:r0 + KC, :], wk_s[...]).astype(bf16)

        _attention_group(g, q_s, k_s, v_s, ctx_s, [functools.partial(k_rows, r0) for r0 in range(0, S, KC)])
        q_proj(half, pair)
        v_proj(half, pair)
        return carry

    lax.fori_loop(0, NG - 1, group, 0)
    _attention_group(NG - 1, q_s, k_s, v_s, ctx_s)

    _tail(x_s, ctx_s, wo_s, w1_s, w2_s, w3_s, w4_s, c_s, wmod_b, h1_s, out_s, o_hbm, osem)


@jax.jit
def pallas_adaLN_cond__compressed_kv_cla__mixer_s_mlp__prompt_kernel(
    A_x: jax.Array,
    A_c_kv: jax.Array,
    A_w_q: jax.Array,
    A_w_uk: jax.Array,
    A_w_uv: jax.Array,
    A_w_o: jax.Array,
    B_x: jax.Array,
    B_w1: jax.Array,
    B_w2: jax.Array,
    B_w3: jax.Array,
    B_w4: jax.Array,
    c: jax.Array,
    w_mod: jax.Array,
):
    del B_x
    x = A_x.reshape(S, M)
    ckv = A_c_kv.reshape(S, DC)
    wo = A_w_o.reshape(H * D, M)

    any_spec = pl.BlockSpec(memory_space=pl.ANY)
    scratch = [
        pltpu.VMEM((S, M), bf16),
        pltpu.VMEM((S // 2, DC), jnp.uint32),
        pltpu.VMEM((2, M, 8, D), jnp.uint32),
        pltpu.VMEM((2, DC, 8, D), jnp.uint32),
        pltpu.VMEM((2, DC, 8, D), jnp.uint32),
        pltpu.VMEM((H * D // 2, M), jnp.uint32),
        pltpu.VMEM((M // 2, M), jnp.uint32),
        pltpu.VMEM((M // 2, M), jnp.uint32),
        pltpu.VMEM((F // 2, M), jnp.uint32),
        pltpu.VMEM((F // 2, M), jnp.uint32),
        pltpu.VMEM((1, M), bf16),
        pltpu.VMEM((M, 2 * M), bf16),
        pltpu.VMEM((M, 4 * M), bf16),
        pltpu.VMEM((S // 2, M), jnp.uint32),
        pltpu.VMEM((M // 2, G * D), jnp.uint32),
        pltpu.VMEM((DC // 2, G * D), jnp.uint32),
        pltpu.VMEM((DC // 2, G * D), jnp.uint32),
        pltpu.VMEM((S // 2, G * D), jnp.uint32),
        pltpu.VMEM((S // 2, G * D), jnp.uint32),
        pltpu.VMEM((S // 2, G * D), jnp.uint32),
        pltpu.VMEM((NG, S // 2, G * D), jnp.uint32),
        pltpu.VMEM((S + 16, M), f32),
        pltpu.VMEM((S, M), bf16),
        pltpu.SemaphoreType.DMA((18 + NX,)),
        pltpu.SemaphoreType.DMA((S // TC,)),
    ]
    out = pl.pallas_call(
        _kernel,
        out_shape=jax.ShapeDtypeStruct((S, M), A_x.dtype),
        in_specs=[any_spec] * 12,
        out_specs=any_spec,
        scratch_shapes=scratch,
        compiler_params=pltpu.CompilerParams(vmem_limit_bytes=126 * 1024 * 1024),
    )(x, ckv, A_w_q, A_w_uk, A_w_uv, wo, B_w1, B_w2, B_w3.T, B_w4, c, w_mod)
    return out.reshape(1, S, M)
```

```python
import functools
import math

import jax
import jax.numpy as jnp
import numpy as np
from jax import lax
from jax.experimental import pallas as pl
from jax.experimental.pallas import tpu as pltpu

S = 2048
M = 640
H = 32
D = 128
DC = 512
F = 1728
G = 2
NG = H // G
R = 128
TC = 256
TIE = 6
LA = 1
ORDER = 0
LC = 128
KC = 1024
XS = (384, 1152)
PEND = 2
EPS = 1e-5
NEG = -1e9
QSCALE = float(D ** -0.5 * math.log2(math.e))

f32 = jnp.float32
bf16 = jnp.bfloat16
_NT = (((1,), (1,)), ((), ()))


def _dot(a, b):
    return jnp.dot(a, b, preferred_element_type=f32)


def _recip(x):
    r = pltpu.reciprocal(x, approx=True)
    r = r * (2.0 - x * r)
    return r * (2.0 - x * r)


def _layernorm(x):
    mu = jnp.mean(x, axis=-1, keepdims=True)
    xc = x - mu
    var = jnp.mean(xc * xc, axis=-1, keepdims=True)
    return xc * lax.rsqrt(var + EPS)


def _gelu(x):
    c = math.sqrt(2.0 / math.pi)
    return 0.5 * x * (1.0 + jnp.tanh(c * (x + 0.044715 * (x * x * x))))


def _relayout(w_raw, half, kdim, pair, dst_ref):
    w = w_raw.at[half].reshape(kdim * 8, D)
    for p in range(G // 2):
        x = w[pl.ds(pair + p, kdim, stride=8), :]
        lo = pltpu.bitcast(x << 16, f32).astype(bf16)
        hi = pltpu.bitcast(x & jnp.uint32(0xFFFF0000), f32).astype(bf16)
        dst_ref[:, (2 * p) * D:(2 * p + 1) * D] = lo
        dst_ref[:, (2 * p + 1) * D:(2 * p + 2) * D] = hi


def _attention_group(g, q_s, k_s, v_s, ctx_s, fillers=()):
    nstrip = S // R
    desc, asc = range(nstrip - 1, -1, -1), range(nstrip)
    orders = [(desc, desc), (asc, desc), (desc, asc), (asc, asc)][ORDER]
    items = [(u, i) for u in range(G) for i in orders[u]]
    n = len(items)
    st = {}
    inv = {}
    row = lax.broadcasted_iota(jnp.int32, (R, R), 0)
    col = lax.broadcasted_iota(jnp.int32, (R, R), 1)
    causal = col <= row

    def scores(t):
        u, i = items[t]
        e = (i + 1) * R
        q = q_s[i * R:(i + 1) * R, u * D:(u + 1) * D]
        s = lax.dot_general(q, k_s[0:e, u * D:(u + 1) * D], _NT, preferred_element_type=f32)
        tiles = [s[:, j * 128:(j + 1) * 128] for j in range(i)]
        tiles.append(jnp.where(causal, s[:, e - R:e], NEG))
        st[t] = {"tiles": tiles}

    def rowmax(t):
        d = st[t]
        m = d["tiles"][0]
        for x in d["tiles"][1:]:
            m = jnp.maximum(m, x)
        mm = jnp.max(m, axis=1, keepdims=True)
        if (t - TIE) in inv:
            mm = mm + 0.0 * inv.pop(t - TIE)
        d["m"] = mm

    def pv(t):
        u, i = items[t]
        d = st[t]
        e = (i + 1) * R
        ps = [jnp.exp2(x - d["m"]) for x in d["tiles"]]
        l = ps[0]
        for x in ps[1:]:
            l = l + x
        d["inv"] = _recip(jnp.sum(l, axis=1, keepdims=True))
        inv[t] = d["inv"]
        p = jnp.concatenate(ps, axis=1).astype(bf16)
        d["o"] = _dot(p, v_s[0:e, u * D:(u + 1) * D])

    def finish(t):
        u, i = items[t]
        d = st.pop(t)
        ctx_s[g, i * R:(i + 1) * R, u * D:(u + 1) * D] = (d["o"] * d["inv"]).astype(bf16)

    fillers = list(fillers)
    for t in range(-LA, n + 1):
        if 0 <= t + LA < n:
            scores(t + LA)
        if t + LA >= n - 1 and fillers:
            fillers.pop(0)()
        if 0 <= t + LA - 1 < n:
            rowmax(t + LA - 1)
        if 0 <= t < n:
            pv(t)
        if 0 <= t - 1 < n:
            finish(t - 1)
    for f in fillers:
        f()


def _tail(x_s, ctx_s, wo_s, w1_s, w2_s, w3_s, w4_s, c_s, wmod_s, h1_s, out_s, o_hbm, osem):
    n = S // TC
    PR = 16
    st = {}
    mod = _modulation(c_s, wmod_s[...])
    ga = mod[:, 0:M]
    sb = mod[:, M:2 * M]
    cb1 = 1.0 + mod[:, 2 * M:3 * M]
    gb = mod[:, 3 * M:4 * M]
    lane = lax.broadcasted_iota(jnp.int32, (1, 128), 1)
    out_copies = []
    pending = []

    def run_pending(k):
        for _ in range(min(k, len(pending))):
            pending.pop(0)()

    def rows(t):
        return slice(t * TC, (t + 1) * TC)

    def oproj(t):
        acc = None
        for g in range(NG):
            part = _dot(ctx_s[g, rows(t), :], wo_s[g * G * D:(g + 1) * G * D, :])
            acc = part if acc is None else acc + part
            run_pending(PEND)
        d = st[t] = {"x1": [], "h": [], "n1": []}

        def piece(j):
            r = slice(j * PR, (j + 1) * PR)
            x1 = x_s[t * TC + j * PR:t * TC + (j + 1) * PR, :].astype(f32) + ga * acc[r]
            h = _layernorm(x1) * cb1 + sb
            d["x1"].append(x1)
            d["h"].append(h)
            d["n1"].append(_layernorm(h).astype(bf16))

        pending.extend(functools.partial(piece, j) for j in range(TC // PR))

    def mm1(t):
        run_pending(len(pending))
        d = st[t]
        h1_s[8 + t * TC:8 + (t + 1) * TC, :] = _gelu(_dot(jnp.concatenate(d.pop("n1"), axis=0), w1_s[...]))

    def mm2(t):
        d = st[t]
        r0 = 8 + t * TC

        def ld(shift, tile):
            return h1_s[r0 + shift:r0 + shift + TC, tile * 128:(tile + 1) * 128]

        c = M // 4
        g = jnp.concatenate([
            ld(-1, 0),
            jnp.where(lane < c - 128, ld(-1, 1), ld(1, 1)),
            jnp.where(lane < 2 * c - 256, ld(1, 2), ld(-2, 2)),
            jnp.where(lane < 3 * c - 384, ld(-2, 3), ld(2, 3)),
            ld(2, 4),
        ], axis=1).astype(bf16)
        hs = _dot(g, w2_s[...])
        d["u"] = []
        d["n2"] = []

        def piece(j):
            u = d["h"][j] + hs[j * PR:(j + 1) * PR]
            d["u"].append(u)
            d["n2"].append(_layernorm(u).astype(bf16))

        pending.extend(functools.partial(piece, j) for j in range(TC // PR))

    def mm3(t):
        d = st[t]
        while len(d["n2"]) < TC // PR:
            run_pending(1)
        a = lax.dot_general(jnp.concatenate(d.pop("n2"), axis=0), w3_s[...], _NT, preferred_element_type=f32)
        d["a"] = _gelu(a).astype(bf16)

    def mm4(t):
        d = st.pop(t)
        y = jnp.concatenate(d["u"], axis=0) + _dot(d["a"], w4_s[...])
        out_s[rows(t), :] = (jnp.concatenate(d["x1"], axis=0) + gb * y).astype(out_s.dtype)
        cp = pltpu.make_async_copy(out_s.at[rows(t), :], o_hbm.at[rows(t), :], osem.at[t])
        cp.start()
        out_copies.append(cp)

    for t in range(-2, n + 1):
        if 0 <= t + 2 < n:
            oproj(t + 2)
        if 0 <= t - 1 < n:
            mm3(t - 1)
        if 0 <= t + 1 < n:
            mm1(t + 1)
        if 0 <= t - 1 < n:
            mm4(t - 1)
        if 0 <= t < n:
            mm2(t)
    for cp in out_copies:
        cp.wait()


def _modulation(c_s, wmod):
    cv = c_s[...].astype(f32)
    sc = (cv * jax.nn.sigmoid(cv)).astype(bf16)
    return _dot(jnp.broadcast_to(sc, (16, M)), wmod)[0:1]


def _kernel(x_hbm, ckv_hbm, wq_hbm, wk_hbm, wv_hbm, wo_hbm, w1_hbm, w2_hbm, w3_hbm, w4_hbm, c_hbm, wmod_hbm,
            o_hbm,
            x_s, ckv_s, wq_raw, wk_raw, wv_raw, wo_s, w1_s, w2_s, w3_s, w4_s, c_s, wmod_a, wmod_b,
            h_s, wq_s, wk_s, wv_s, q_s, k_s, v_s, ctx_s, h1_s, out_s, sems, osem):
    h_s, wq_s, wk_s, wv_s, q_s, k_s, v_s, ctx_s = (r.bitcast(bf16) for r in (h_s, wq_s, wk_s, wv_s, q_s, k_s, v_s, ctx_s))
    u32 = jnp.uint32
    wq32, wk32, wv32 = (w.bitcast(u32) for w in (wq_hbm, wk_hbm, wv_hbm))
    xb = list(zip((0,) + XS, XS + (S,)))
    first = [
        (ckv_hbm.bitcast(u32), ckv_s),
        (wk32.at[:, 0:4, :], wk_raw.at[0, :, 0:4, :]),
        (wv32.at[:, 0:4, :], wv_raw.at[0, :, 0:4, :]),
        (c_hbm, c_s),
        (wmod_hbm.at[:, 0:2 * M], wmod_a),
        (wq32.at[:, 0:4, :], wq_raw.at[0, :, 0:4, :]),
    ] + [(x_hbm.at[a:b, :], x_s.at[a:b, :]) for a, b in xb]
    later = [
        (wk32.at[:, 4:8, :], wk_raw.at[0, :, 4:8, :]),
        (wq32.at[:, 4:8, :], wq_raw.at[0, :, 4:8, :]),
        (wv32.at[:, 4:8, :], wv_raw.at[0, :, 4:8, :]),
        (wk32.at[:, 8:16, :], wk_raw.at[1]),
        (wq32.at[:, 8:16, :], wq_raw.at[1]),
        (wv32.at[:, 8:16, :], wv_raw.at[1]),
    ]
    last = [
        (wo_hbm.bitcast(u32), wo_s),
        (wmod_hbm.at[:, 2 * M:6 * M], wmod_b),
        (w1_hbm.bitcast(u32), w1_s),
        (w2_hbm.bitcast(u32), w2_s),
        (w3_hbm.bitcast(u32), w3_s),
        (w4_hbm.bitcast(u32), w4_s),
    ]
    copies = [pltpu.make_async_copy(src, dst, sems.at[i]) for i, (src, dst) in enumerate(first + later + last)]
    for cp in copies:
        cp.start()
    cp_ckv, cp_wk0, cp_wv0, cp_c, cp_wma, cp_wq0 = copies[:6]
    cp_x = copies[6:len(first)]
    cp_later = copies[len(first):len(first) + len(later)]
    cp_last = copies[len(first) + len(later):]
    ckv_s, wo_s, w1_s, w2_s, w3_s, w4_s, h_s, wq_s, wk_s, wv_s, q_s, k_s, v_s, ctx_s = (
        r.bitcast(bf16) for r in (ckv_s, wo_s, w1_s, w2_s, w3_s, w4_s, h_s, wq_s, wk_s, wv_s, q_s, k_s, v_s, ctx_s))

    def k_proj(half, pair):
        _relayout(wk_raw, half, DC, pair, wk_s)
        k_s[...] = _dot(ckv_s[...], wk_s[...]).astype(bf16)

    def v_proj(half, pair):
        _relayout(wv_raw, half, DC, pair, wv_s)
        v_s[...] = _dot(ckv_s[...], wv_s[...]).astype(bf16)

    def q_proj(half, pair):
        _relayout(wq_raw, half, M, pair, wq_s)
        q_s[...] = (_dot(h_s[...], wq_s[...]) * QSCALE).astype(bf16)

    h1_s[0:8, :] = jnp.zeros((8, M), f32)
    h1_s[8 + S:16 + S, :] = jnp.zeros((8, M), f32)

    cp_ckv.wait()
    cp_wk0.wait()
    k_proj(0, 0)
    cp_wv0.wait()
    v_proj(0, 0)
    cp_c.wait()
    cp_wma.wait()
    cp_wq0.wait()
    mod = _modulation(c_s, wmod_a[...])
    sa = mod[:, 0:M]
    ca1 = 1.0 + mod[:, M:2 * M]
    _relayout(wq_raw, 0, M, 0, wq_s)
    def ln_rows(r0):
        xi = x_s[r0:r0 + LC, :].astype(f32)
        h_s[r0:r0 + LC, :] = (_layernorm(xi) * ca1 + sa).astype(bf16)

    for cp, (a, b) in zip(cp_x, xb):
        cp.wait()
        starts = list(range(a, b, LC))
        ln_rows(starts[0])
        for i, r0 in enumerate(starts):
            if i + 1 < len(starts):
                ln_rows(starts[i + 1])
            q_s[r0:r0 + LC, :] = (_dot(h_s[r0:r0 + LC, :], wq_s[...]) * QSCALE).astype(bf16)

    def group(g, carry):
        @pl.when(g == 2)
        def _():
            for cp in cp_later:
                cp.wait()

        @pl.when(g == 8)
        def _():
            for cp in cp_last:
                cp.wait()

        half = (g + 1) // (NG // 2)
        pair = ((g + 1) % (NG // 2)) * (G // 2)
        _relayout(wk_raw, half, DC, pair, wk_s)

        def k_rows(r0):
            k_s[r0:r0 + KC, :] = _dot(ckv_s[r0:r0 + KC, :], wk_s[...]).astype(bf16)

        _attention_group(g, q_s, k_s, v_s, ctx_s, [functools.partial(k_rows, r0) for r0 in range(0, S, KC)])
        q_proj(half, pair)
        v_proj(half, pair)
        return carry

    lax.fori_loop(0, NG - 1, group, 0)
    _attention_group(NG - 1, q_s, k_s, v_s, ctx_s)

    _tail(x_s, ctx_s, wo_s, w1_s, w2_s, w3_s, w4_s, c_s, wmod_b, h1_s, out_s, o_hbm, osem)


@jax.jit
def pallas_adaLN_cond__compressed_kv_cla__mixer_s_mlp__prompt_kernel(
    A_x: jax.Array,
    A_c_kv: jax.Array,
    A_w_q: jax.Array,
    A_w_uk: jax.Array,
    A_w_uv: jax.Array,
    A_w_o: jax.Array,
    B_x: jax.Array,
    B_w1: jax.Array,
    B_w2: jax.Array,
    B_w3: jax.Array,
    B_w4: jax.Array,
    c: jax.Array,
    w_mod: jax.Array,
):
    del B_x
    x = A_x.reshape(S, M)
    ckv = A_c_kv.reshape(S, DC)
    wo = A_w_o.reshape(H * D, M)

    any_spec = pl.BlockSpec(memory_space=pl.ANY)
    scratch = [
        pltpu.VMEM((S, M), bf16),
        pltpu.VMEM((S // 2, DC), jnp.uint32),
        pltpu.VMEM((2, M, 8, D), jnp.uint32),
        pltpu.VMEM((2, DC, 8, D), jnp.uint32),
        pltpu.VMEM((2, DC, 8, D), jnp.uint32),
        pltpu.VMEM((H * D // 2, M), jnp.uint32),
        pltpu.VMEM((M // 2, M), jnp.uint32),
        pltpu.VMEM((M // 2, M), jnp.uint32),
        pltpu.VMEM((F // 2, M), jnp.uint32),
        pltpu.VMEM((F // 2, M), jnp.uint32),
        pltpu.VMEM((1, M), bf16),
        pltpu.VMEM((M, 2 * M), bf16),
        pltpu.VMEM((M, 4 * M), bf16),
        pltpu.VMEM((S // 2, M), jnp.uint32),
        pltpu.VMEM((M // 2, G * D), jnp.uint32),
        pltpu.VMEM((DC // 2, G * D), jnp.uint32),
        pltpu.VMEM((DC // 2, G * D), jnp.uint32),
        pltpu.VMEM((S // 2, G * D), jnp.uint32),
        pltpu.VMEM((S // 2, G * D), jnp.uint32),
        pltpu.VMEM((S // 2, G * D), jnp.uint32),
        pltpu.VMEM((NG, S // 2, G * D), jnp.uint32),
        pltpu.VMEM((S + 16, M), f32),
        pltpu.VMEM((S, M), bf16),
        pltpu.SemaphoreType.DMA((19 + len(XS),)),
        pltpu.SemaphoreType.DMA((S // TC,)),
    ]
    out = pl.pallas_call(
        _kernel,
        out_shape=jax.ShapeDtypeStruct((S, M), A_x.dtype),
        in_specs=[any_spec] * 12,
        out_specs=any_spec,
        scratch_shapes=scratch,
        compiler_params=pltpu.CompilerParams(vmem_limit_bytes=126 * 1024 * 1024),
    )(x, ckv, A_w_q, A_w_uk, A_w_uv, wo, B_w1, B_w2, B_w3.T, B_w4, c, w_mod)
    return out.reshape(1, S, M)
```

```python
import functools
import math

import jax
import jax.numpy as jnp
from jax import lax
from jax.experimental import pallas as pl
from jax.experimental.pallas import tpu as pltpu

S = 2048
M = 640
H = 32
D = 128
DC = 512
F = 1728
G = 2
assert G == 2
NG = H // G
R = 128
TC = 256
TIE = 6
LA = 1
LC = 128
KC = 1024
XS = (384, 1152)
PEND = 2
EPS = 1e-5
NEG = -1e9
QSCALE = float(D ** -0.5 * math.log2(math.e))

f32 = jnp.float32
bf16 = jnp.bfloat16
_NT = (((1,), (1,)), ((), ()))


def _dot(a, b):
    return jnp.dot(a, b, preferred_element_type=f32)


def _recip(x):
    r = pltpu.reciprocal(x, approx=True)
    r = r * (2.0 - x * r)
    return r * (2.0 - x * r)


def _layernorm(x):
    mu = jnp.mean(x, axis=-1, keepdims=True)
    xc = x - mu
    var = jnp.mean(xc * xc, axis=-1, keepdims=True)
    return xc * lax.rsqrt(var + EPS)


def _gelu(x):
    c = math.sqrt(2.0 / math.pi)
    return 0.5 * x * (1.0 + jnp.tanh(c * (x + 0.044715 * (x * x * x))))


def _relayout(w_raw, block, kdim, pair, dst_ref):
    w = w_raw.at[block].reshape(kdim * 8, D)
    for p in range(G // 2):
        x = w[pl.ds(pair + p, kdim, stride=8), :]
        lo = pltpu.bitcast(x << 16, f32).astype(bf16)
        hi = pltpu.bitcast(x & jnp.uint32(0xFFFF0000), f32).astype(bf16)
        dst_ref[:, (2 * p) * D:(2 * p + 1) * D] = lo
        dst_ref[:, (2 * p + 1) * D:(2 * p + 2) * D] = hi


def _attention_group(g, q_s, k_s, v_s, ctx_s, fillers=()):
    nstrip = S // R
    items = [(u, i) for u in range(G) for i in range(nstrip - 1, -1, -1)]
    n = len(items)
    st = {}
    inv = {}
    row = lax.broadcasted_iota(jnp.int32, (R, R), 0)
    col = lax.broadcasted_iota(jnp.int32, (R, R), 1)
    causal = col <= row

    def scores(t):
        u, i = items[t]
        e = (i + 1) * R
        q = q_s[i * R:(i + 1) * R, u * D:(u + 1) * D]
        s = lax.dot_general(q, k_s[0:e, u * D:(u + 1) * D], _NT, preferred_element_type=f32)
        tiles = [s[:, j * 128:(j + 1) * 128] for j in range(i)]
        tiles.append(jnp.where(causal, s[:, e - R:e], NEG))
        st[t] = {"tiles": tiles}

    def rowmax(t):
        d = st[t]
        m = d["tiles"][0]
        for x in d["tiles"][1:]:
            m = jnp.maximum(m, x)
        mm = jnp.max(m, axis=1, keepdims=True)
        if (t - TIE) in inv:
            mm = mm + 0.0 * inv.pop(t - TIE)
        d["m"] = mm

    def pv(t):
        u, i = items[t]
        d = st[t]
        e = (i + 1) * R
        ps = [jnp.exp2(x - d["m"]) for x in d["tiles"]]
        l = ps[0]
        for x in ps[1:]:
            l = l + x
        d["inv"] = _recip(jnp.sum(l, axis=1, keepdims=True))
        inv[t] = d["inv"]
        p = jnp.concatenate(ps, axis=1).astype(bf16)
        d["o"] = _dot(p, v_s[0:e, u * D:(u + 1) * D])

    def finish(t):
        u, i = items[t]
        d = st.pop(t)
        ctx_s[g, i * R:(i + 1) * R, u * D:(u + 1) * D] = (d["o"] * d["inv"]).astype(bf16)

    fillers = list(fillers)
    for t in range(-LA, n + 1):
        if 0 <= t + LA < n:
            scores(t + LA)
        if t + LA >= n - 1 and fillers:
            fillers.pop(0)()
        if 0 <= t + LA - 1 < n:
            rowmax(t + LA - 1)
        if 0 <= t < n:
            pv(t)
        if 0 <= t - 1 < n:
            finish(t - 1)
    for f in fillers:
        f()


def _tail(x_s, ctx_s, wo_s, w1_s, w2_s, w3_s, w4_s, c_s, wmod_s, h1_s, out_s, o_hbm, osem):
    n = S // TC
    PR = 16
    st = {}
    mod = _modulation(c_s, wmod_s[...])
    ga = mod[:, 0:M]
    sb = mod[:, M:2 * M]
    cb1 = 1.0 + mod[:, 2 * M:3 * M]
    gb = mod[:, 3 * M:4 * M]
    lane = lax.broadcasted_iota(jnp.int32, (1, 128), 1)
    out_copies = []
    pending = []

    def run_pending(k):
        for _ in range(min(k, len(pending))):
            pending.pop(0)()

    def rows(t):
        return slice(t * TC, (t + 1) * TC)

    def oproj(t):
        acc = None
        for g in range(NG):
            part = _dot(ctx_s[g, rows(t), :], wo_s[g * G * D:(g + 1) * G * D, :])
            acc = part if acc is None else acc + part
            run_pending(PEND)
        d = st[t] = {"x1": [], "h": [], "n1": []}

        def piece(j):
            r = slice(j * PR, (j + 1) * PR)
            x1 = x_s[t * TC + j * PR:t * TC + (j + 1) * PR, :].astype(f32) + ga * acc[r]
            h = _layernorm(x1) * cb1 + sb
            d["x1"].append(x1)
            d["h"].append(h)
            d["n1"].append(_layernorm(h).astype(bf16))

        pending.extend(functools.partial(piece, j) for j in range(TC // PR))

    def mm1(t):
        run_pending(len(pending))
        d = st[t]
        h1_s[8 + t * TC:8 + (t + 1) * TC, :] = _gelu(_dot(jnp.concatenate(d.pop("n1"), axis=0), w1_s[...]))

    def mm2(t):
        d = st[t]
        r0 = 8 + t * TC

        def ld(shift, tile):
            return h1_s[r0 + shift:r0 + shift + TC, tile * 128:(tile + 1) * 128]

        c = M // 4
        g = jnp.concatenate([
            ld(-1, 0),
            jnp.where(lane < c - 128, ld(-1, 1), ld(1, 1)),
            jnp.where(lane < 2 * c - 256, ld(1, 2), ld(-2, 2)),
            jnp.where(lane < 3 * c - 384, ld(-2, 3), ld(2, 3)),
            ld(2, 4),
        ], axis=1).astype(bf16)
        hs = _dot(g, w2_s[...])
        d["u"] = []
        d["n2"] = []

        def piece(j):
            u = d["h"][j] + hs[j * PR:(j + 1) * PR]
            d["u"].append(u)
            d["n2"].append(_layernorm(u).astype(bf16))

        pending.extend(functools.partial(piece, j) for j in range(TC // PR))

    def mm3(t):
        d = st[t]
        while len(d["n2"]) < TC // PR:
            run_pending(1)
        a = lax.dot_general(jnp.concatenate(d.pop("n2"), axis=0), w3_s[...], _NT, preferred_element_type=f32)
        d["a"] = _gelu(a).astype(bf16)

    def mm4(t):
        d = st.pop(t)
        y = jnp.concatenate(d["u"], axis=0) + _dot(d["a"], w4_s[...])
        out_s[rows(t), :] = (jnp.concatenate(d["x1"], axis=0) + gb * y).astype(out_s.dtype)
        cp = pltpu.make_async_copy(out_s.at[rows(t), :], o_hbm.at[rows(t), :], osem.at[t])
        cp.start()
        out_copies.append(cp)

    for t in range(-2, n + 1):
        if 0 <= t + 2 < n:
            oproj(t + 2)
        if 0 <= t - 1 < n:
            mm3(t - 1)
        if 0 <= t + 1 < n:
            mm1(t + 1)
        if 0 <= t - 1 < n:
            mm4(t - 1)
        if 0 <= t < n:
            mm2(t)
    for cp in out_copies:
        cp.wait()


def _modulation(c_s, wmod):
    cv = c_s[...].astype(f32)
    sc = (cv * jax.nn.sigmoid(cv)).astype(bf16)
    return _dot(jnp.broadcast_to(sc, (16, M)), wmod)[0:1]


def _kernel(x_hbm, ckv_hbm, wq_hbm, wk_hbm, wv_hbm, wo_hbm, w1_hbm, w2_hbm, w3_hbm, w4_hbm, c_hbm, wmod_hbm,
            o_hbm,
            x_s, ckv_s, wq_raw, wk_raw, wv_raw, wo_s, w1_s, w2_s, w3_s, w4_s, c_s, wmod_a, wmod_b,
            h_s, wq_s, wk_s, wv_s, q_s, k_s, v_s, ctx_s, h1_s, out_s, sems, osem):
    h_s, wq_s, wk_s, wv_s, q_s, k_s, v_s, ctx_s = (r.bitcast(bf16) for r in (h_s, wq_s, wk_s, wv_s, q_s, k_s, v_s, ctx_s))
    u32 = jnp.uint32
    wq32, wk32, wv32 = (w.bitcast(u32) for w in (wq_hbm, wk_hbm, wv_hbm))
    xb = list(zip((0,) + XS, XS + (S,)))
    first = [
        (ckv_hbm.bitcast(u32), ckv_s),
        (wk32.at[:, 0:4, :], wk_raw.at[0, :, 0:4, :]),
        (wv32.at[:, 0:4, :], wv_raw.at[0, :, 0:4, :]),
        (c_hbm, c_s),
        (wmod_hbm.at[:, 0:2 * M], wmod_a),
        (wq32.at[:, 0:4, :], wq_raw.at[0, :, 0:4, :]),
    ] + [(x_hbm.at[a:b, :], x_s.at[a:b, :]) for a, b in xb]
    later = [(w32.at[:, 4 * q:4 * q + 4, :], raw.at[q, :, 0:4, :])
             for q in range(1, 4) for w32, raw in ((wk32, wk_raw), (wq32, wq_raw), (wv32, wv_raw))]
    last = [
        (wo_hbm.bitcast(u32), wo_s),
        (wmod_hbm.at[:, 2 * M:6 * M], wmod_b),
        (w1_hbm.bitcast(u32), w1_s),
        (w2_hbm.bitcast(u32), w2_s),
        (w3_hbm.bitcast(u32), w3_s),
        (w4_hbm.bitcast(u32), w4_s),
    ]
    copies = [pltpu.make_async_copy(src, dst, sems.at[i]) for i, (src, dst) in enumerate(first + later + last)]
    for cp in copies:
        cp.start()
    cp_ckv, cp_wk0, cp_wv0, cp_c, cp_wma, cp_wq0 = copies[:6]
    cp_x = copies[6:len(first)]
    cp_later = copies[len(first):len(first) + len(later)]
    cp_last = copies[len(first) + len(later):]
    ckv_s, wo_s, w1_s, w2_s, w3_s, w4_s, h_s, wq_s, wk_s, wv_s, q_s, k_s, v_s, ctx_s = (
        r.bitcast(bf16) for r in (ckv_s, wo_s, w1_s, w2_s, w3_s, w4_s, h_s, wq_s, wk_s, wv_s, q_s, k_s, v_s, ctx_s))

    def k_proj(block, pair):
        _relayout(wk_raw, block, DC, pair, wk_s)
        k_s[...] = _dot(ckv_s[...], wk_s[...]).astype(bf16)

    def v_proj(block, pair):
        _relayout(wv_raw, block, DC, pair, wv_s)
        v_s[...] = _dot(ckv_s[...], wv_s[...]).astype(bf16)

    def q_proj(block, pair):
        _relayout(wq_raw, block, M, pair, wq_s)
        q_s[...] = (_dot(h_s[...], wq_s[...]) * QSCALE).astype(bf16)

    h1_s[0:8, :] = jnp.zeros((8, M), f32)
    h1_s[8 + S:16 + S, :] = jnp.zeros((8, M), f32)

    cp_ckv.wait()
    cp_wk0.wait()
    k_proj(0, 0)
    cp_wv0.wait()
    v_proj(0, 0)
    cp_c.wait()
    cp_wma.wait()
    cp_wq0.wait()
    mod = _modulation(c_s, wmod_a[...])
    sa = mod[:, 0:M]
    ca1 = 1.0 + mod[:, M:2 * M]
    _relayout(wq_raw, 0, M, 0, wq_s)
    def ln_rows(r0):
        xi = x_s[r0:r0 + LC, :].astype(f32)
        h_s[r0:r0 + LC, :] = (_layernorm(xi) * ca1 + sa).astype(bf16)

    for cp, (a, b) in zip(cp_x, xb):
        cp.wait()
        starts = list(range(a, b, LC))
        ln_rows(starts[0])
        for i, r0 in enumerate(starts):
            if i + 1 < len(starts):
                ln_rows(starts[i + 1])
            q_s[r0:r0 + LC, :] = (_dot(h_s[r0:r0 + LC, :], wq_s[...]) * QSCALE).astype(bf16)

    def group(g, carry):
        @pl.when(g == 2)
        def _():
            for cp in cp_later:
                cp.wait()

        @pl.when(g == 8)
        def _():
            for cp in cp_last:
                cp.wait()

        block = (g + 1) // 4
        pair = (g + 1) % 4
        _relayout(wk_raw, block, DC, pair, wk_s)

        def k_rows(r0):
            k_s[r0:r0 + KC, :] = _dot(ckv_s[r0:r0 + KC, :], wk_s[...]).astype(bf16)

        _attention_group(g, q_s, k_s, v_s, ctx_s, [functools.partial(k_rows, r0) for r0 in range(0, S, KC)])
        q_proj(block, pair)
        v_proj(block, pair)
        return carry

    lax.fori_loop(0, NG - 1, group, 0)
    _attention_group(NG - 1, q_s, k_s, v_s, ctx_s)

    _tail(x_s, ctx_s, wo_s, w1_s, w2_s, w3_s, w4_s, c_s, wmod_b, h1_s, out_s, o_hbm, osem)


@jax.jit
def pallas_adaLN_cond__compressed_kv_cla__mixer_s_mlp__prompt_kernel(
    A_x: jax.Array,
    A_c_kv: jax.Array,
    A_w_q: jax.Array,
    A_w_uk: jax.Array,
    A_w_uv: jax.Array,
    A_w_o: jax.Array,
    B_x: jax.Array,
    B_w1: jax.Array,
    B_w2: jax.Array,
    B_w3: jax.Array,
    B_w4: jax.Array,
    c: jax.Array,
    w_mod: jax.Array,
):
    del B_x
    x = A_x.reshape(S, M)
    ckv = A_c_kv.reshape(S, DC)
    wo = A_w_o.reshape(H * D, M)

    any_spec = pl.BlockSpec(memory_space=pl.ANY)
    scratch = [
        pltpu.VMEM((S, M), bf16),
        pltpu.VMEM((S // 2, DC), jnp.uint32),
        pltpu.VMEM((4, M, 8, D), jnp.uint32),
        pltpu.VMEM((4, DC, 8, D), jnp.uint32),
        pltpu.VMEM((4, DC, 8, D), jnp.uint32),
        pltpu.VMEM((H * D // 2, M), jnp.uint32),
        pltpu.VMEM((M // 2, M), jnp.uint32),
        pltpu.VMEM((M // 2, M), jnp.uint32),
        pltpu.VMEM((F // 2, M), jnp.uint32),
        pltpu.VMEM((F // 2, M), jnp.uint32),
        pltpu.VMEM((1, M), bf16),
        pltpu.VMEM((M, 2 * M), bf16),
        pltpu.VMEM((M, 4 * M), bf16),
        pltpu.VMEM((S // 2, M), jnp.uint32),
        pltpu.VMEM((M // 2, G * D), jnp.uint32),
        pltpu.VMEM((DC // 2, G * D), jnp.uint32),
        pltpu.VMEM((DC // 2, G * D), jnp.uint32),
        pltpu.VMEM((S // 2, G * D), jnp.uint32),
        pltpu.VMEM((S // 2, G * D), jnp.uint32),
        pltpu.VMEM((S // 2, G * D), jnp.uint32),
        pltpu.VMEM((NG, S // 2, G * D), jnp.uint32),
        pltpu.VMEM((S + 16, M), f32),
        pltpu.VMEM((S, M), bf16),
        pltpu.SemaphoreType.DMA((22 + len(XS),)),
        pltpu.SemaphoreType.DMA((S // TC,)),
    ]
    out = pl.pallas_call(
        _kernel,
        out_shape=jax.ShapeDtypeStruct((S, M), A_x.dtype),
        in_specs=[any_spec] * 12,
        out_specs=any_spec,
        scratch_shapes=scratch,
        compiler_params=pltpu.CompilerParams(vmem_limit_bytes=126 * 1024 * 1024),
    )(x, ckv, A_w_q, A_w_uk, A_w_uv, wo, B_w1, B_w2, B_w3.T, B_w4, c, w_mod)
    return out.reshape(1, S, M)
```

```python
import functools
import math

import jax
import jax.numpy as jnp
from jax import lax
from jax.experimental import pallas as pl
from jax.experimental.pallas import tpu as pltpu

S = 2048
M = 640
H = 32
D = 128
DC = 512
F = 1728
G = 2
assert G == 2
NG = H // G
R = 128
TC = 256
TIE = 6
LA = 1
LC = 128
KC = 1024
XS = (384, 1152)
PEND = 2
EPS = 1e-5
NEG = -1e9
QSCALE = float(D ** -0.5 * math.log2(math.e))

f32 = jnp.float32
bf16 = jnp.bfloat16
_NT = (((1,), (1,)), ((), ()))


def _dot(a, b):
    return jnp.dot(a, b, preferred_element_type=f32)


def _recip(x):
    r = pltpu.reciprocal(x, approx=True)
    r = r * (2.0 - x * r)
    return r * (2.0 - x * r)


def _layernorm(x):
    mu = jnp.mean(x, axis=-1, keepdims=True)
    xc = x - mu
    var = jnp.mean(xc * xc, axis=-1, keepdims=True)
    return xc * lax.rsqrt(var + EPS)


def _gelu(x):
    c = math.sqrt(2.0 / math.pi)
    return 0.5 * x * (1.0 + jnp.tanh(c * (x + 0.044715 * (x * x * x))))


def _relayout(w_raw, block, kdim, pair, dst_ref):
    w = w_raw.at[block].reshape(kdim * 8, D)
    for p in range(G // 2):
        x = w[pl.ds(pair + p, kdim, stride=8), :]
        lo = pltpu.bitcast(x << 16, f32).astype(bf16)
        hi = pltpu.bitcast(x & jnp.uint32(0xFFFF0000), f32).astype(bf16)
        dst_ref[:, (2 * p) * D:(2 * p + 1) * D] = lo
        dst_ref[:, (2 * p + 1) * D:(2 * p + 2) * D] = hi


def _attention_group(g, q_s, k_s, v_s, ctx_s, fillers=()):
    nstrip = S // R
    items = [(u, i) for u in range(G) for i in range(nstrip - 1, -1, -1)]
    n = len(items)
    st = {}
    inv = {}
    row = lax.broadcasted_iota(jnp.int32, (R, R), 0)
    col = lax.broadcasted_iota(jnp.int32, (R, R), 1)
    causal = col <= row

    def scores(t):
        u, i = items[t]
        e = (i + 1) * R
        q = q_s[i * R:(i + 1) * R, u * D:(u + 1) * D]
        s = lax.dot_general(q, k_s[0:e, u * D:(u + 1) * D], _NT, preferred_element_type=f32)
        tiles = [s[:, j * 128:(j + 1) * 128] for j in range(i)]
        tiles.append(jnp.where(causal, s[:, e - R:e], NEG))
        st[t] = {"tiles": tiles}

    def rowmax(t):
        d = st[t]
        m = d["tiles"][0]
        for x in d["tiles"][1:]:
            m = jnp.maximum(m, x)
        mm = jnp.max(m, axis=1, keepdims=True)
        if (t - TIE) in inv:
            mm = mm + 0.0 * inv.pop(t - TIE)
        d["m"] = mm

    def pv(t):
        u, i = items[t]
        d = st[t]
        e = (i + 1) * R
        ps = [jnp.exp2(x - d["m"]) for x in d["tiles"]]
        l = ps[0]
        for x in ps[1:]:
            l = l + x
        d["inv"] = _recip(jnp.sum(l, axis=1, keepdims=True))
        inv[t] = d["inv"]
        p = jnp.concatenate(ps, axis=1).astype(bf16)
        d["o"] = _dot(p, v_s[0:e, u * D:(u + 1) * D])

    def finish(t):
        u, i = items[t]
        d = st.pop(t)
        ctx_s[g, i * R:(i + 1) * R, u * D:(u + 1) * D] = (d["o"] * d["inv"]).astype(bf16)

    fillers = list(fillers)
    for t in range(-LA, n + 1):
        if 0 <= t + LA < n:
            scores(t + LA)
        if t + LA >= n - 1 and fillers:
            fillers.pop(0)()
        if 0 <= t + LA - 1 < n:
            rowmax(t + LA - 1)
        if 0 <= t < n:
            pv(t)
        if 0 <= t - 1 < n:
            finish(t - 1)
    for f in fillers:
        f()


def _tail(x_s, ctx_s, wo_s, w1_s, w2_s, w3_s, w4_s, c_s, wmod_s, h1_s, out_s, o_hbm, osem):
    n = S // TC
    PR = 16
    st = {}
    mod = _modulation(c_s, wmod_s[...])
    ga = mod[:, 0:M]
    sb = mod[:, M:2 * M]
    cb1 = 1.0 + mod[:, 2 * M:3 * M]
    gb = mod[:, 3 * M:4 * M]
    lane = lax.broadcasted_iota(jnp.int32, (1, 128), 1)
    out_copies = []
    pending = []

    def run_pending(k):
        for _ in range(min(k, len(pending))):
            pending.pop(0)()

    def rows(t):
        return slice(t * TC, (t + 1) * TC)

    def oproj(t):
        accs = []
        for c0 in range(0, M, 128):
            acc = None
            for g in range(0, NG, 2):
                lhs = jnp.concatenate([ctx_s[g + j, rows(t), :] for j in range(2)], axis=1)
                part = _dot(lhs, wo_s[g * G * D:(g + 2) * G * D, c0:c0 + 128])
                acc = part if acc is None else acc + part
            accs.append(acc)
            run_pending(8)
        acc = jnp.concatenate(accs, axis=1)
        d = st[t] = {"x1": [], "h": [], "n1": []}

        def piece(j):
            r = slice(j * PR, (j + 1) * PR)
            x1 = x_s[t * TC + j * PR:t * TC + (j + 1) * PR, :].astype(f32) + ga * acc[r]
            h = _layernorm(x1) * cb1 + sb
            d["x1"].append(x1)
            d["h"].append(h)
            d["n1"].append(_layernorm(h).astype(bf16))

        pending.extend(functools.partial(piece, j) for j in range(TC // PR))

    def mm1(t):
        run_pending(len(pending))
        d = st[t]
        h1_s[8 + t * TC:8 + (t + 1) * TC, :] = _gelu(_dot(jnp.concatenate(d.pop("n1"), axis=0), w1_s[...]))

    def mm2(t):
        d = st[t]
        r0 = 8 + t * TC

        def ld(shift, tile):
            return h1_s[r0 + shift:r0 + shift + TC, tile * 128:(tile + 1) * 128]

        c = M // 4
        g = jnp.concatenate([
            ld(-1, 0),
            jnp.where(lane < c - 128, ld(-1, 1), ld(1, 1)),
            jnp.where(lane < 2 * c - 256, ld(1, 2), ld(-2, 2)),
            jnp.where(lane < 3 * c - 384, ld(-2, 3), ld(2, 3)),
            ld(2, 4),
        ], axis=1).astype(bf16)
        hs = _dot(g, w2_s[...])
        d["u"] = []
        d["n2"] = []

        def piece(j):
            u = d["h"][j] + hs[j * PR:(j + 1) * PR]
            d["u"].append(u)
            d["n2"].append(_layernorm(u).astype(bf16))

        pending.extend(functools.partial(piece, j) for j in range(TC // PR))

    def mm3(t):
        d = st[t]
        while len(d["n2"]) < TC // PR:
            run_pending(1)
        a = lax.dot_general(jnp.concatenate(d.pop("n2"), axis=0), w3_s[...], _NT, preferred_element_type=f32)
        d["a"] = _gelu(a).astype(bf16)

    def mm4(t):
        d = st.pop(t)
        y = jnp.concatenate(d["u"], axis=0) + _dot(d["a"], w4_s[...])
        out_s[rows(t), :] = (jnp.concatenate(d["x1"], axis=0) + gb * y).astype(out_s.dtype)
        cp = pltpu.make_async_copy(out_s.at[rows(t), :], o_hbm.at[rows(t), :], osem.at[t])
        cp.start()
        out_copies.append(cp)

    for t in range(-2, n + 1):
        if 0 <= t + 2 < n:
            oproj(t + 2)
        if 0 <= t - 1 < n:
            mm3(t - 1)
        if 0 <= t + 1 < n:
            mm1(t + 1)
        if 0 <= t - 1 < n:
            mm4(t - 1)
        if 0 <= t < n:
            mm2(t)
    for cp in out_copies:
        cp.wait()


def _modulation(c_s, wmod):
    cv = c_s[...].astype(f32)
    sc = (cv * jax.nn.sigmoid(cv)).astype(bf16)
    return _dot(jnp.broadcast_to(sc, (16, M)), wmod)[0:1]


def _kernel(x_hbm, ckv_hbm, wq_hbm, wk_hbm, wv_hbm, wo_hbm, w1_hbm, w2_hbm, w3_hbm, w4_hbm, c_hbm, wmod_hbm,
            o_hbm,
            x_s, ckv_s, wq_raw, wk_raw, wv_raw, wo_s, w1_s, w2_s, w3_s, w4_s, c_s, wmod_a, wmod_b,
            h_s, wq_s, wk_s, wv_s, q_s, k_s, v_s, ctx_s, h1_s, out_s, sems, osem):
    h_s, wq_s, wk_s, wv_s, q_s, k_s, v_s, ctx_s = (r.bitcast(bf16) for r in (h_s, wq_s, wk_s, wv_s, q_s, k_s, v_s, ctx_s))
    u32 = jnp.uint32
    wq32, wk32, wv32 = (w.bitcast(u32) for w in (wq_hbm, wk_hbm, wv_hbm))
    xb = list(zip((0,) + XS, XS + (S,)))
    first = [
        (ckv_hbm.bitcast(u32), ckv_s),
        (wk32.at[:, 0:4, :], wk_raw.at[0, :, 0:4, :]),
        (wv32.at[:, 0:4, :], wv_raw.at[0, :, 0:4, :]),
        (c_hbm, c_s),
        (wmod_hbm.at[:, 0:2 * M], wmod_a),
        (wq32.at[:, 0:4, :], wq_raw.at[0, :, 0:4, :]),
    ] + [(x_hbm.at[a:b, :], x_s.at[a:b, :]) for a, b in xb]
    later = [(w32.at[:, 4 * q:4 * q + 4, :], raw.at[q, :, 0:4, :])
             for q in range(1, 4) for w32, raw in ((wk32, wk_raw), (wq32, wq_raw), (wv32, wv_raw))]
    last = [
        (wo_hbm.bitcast(u32), wo_s),
        (wmod_hbm.at[:, 2 * M:6 * M], wmod_b),
        (w1_hbm.bitcast(u32), w1_s),
        (w2_hbm.bitcast(u32), w2_s),
        (w3_hbm.bitcast(u32), w3_s),
        (w4_hbm.bitcast(u32), w4_s),
    ]
    copies = [pltpu.make_async_copy(src, dst, sems.at[i]) for i, (src, dst) in enumerate(first + later + last)]
    for cp in copies:
        cp.start()
    cp_ckv, cp_wk0, cp_wv0, cp_c, cp_wma, cp_wq0 = copies[:6]
    cp_x = copies[6:len(first)]
    cp_later = copies[len(first):len(first) + len(later)]
    cp_last = copies[len(first) + len(later):]
    ckv_s, wo_s, w1_s, w2_s, w3_s, w4_s, h_s, wq_s, wk_s, wv_s, q_s, k_s, v_s, ctx_s = (
        r.bitcast(bf16) for r in (ckv_s, wo_s, w1_s, w2_s, w3_s, w4_s, h_s, wq_s, wk_s, wv_s, q_s, k_s, v_s, ctx_s))

    def k_proj(block, pair):
        _relayout(wk_raw, block, DC, pair, wk_s)
        k_s[...] = _dot(ckv_s[...], wk_s[...]).astype(bf16)

    def v_proj(block, pair):
        _relayout(wv_raw, block, DC, pair, wv_s)
        v_s[...] = _dot(ckv_s[...], wv_s[...]).astype(bf16)

    def q_proj(block, pair):
        _relayout(wq_raw, block, M, pair, wq_s)
        q_s[...] = (_dot(h_s[...], wq_s[...]) * QSCALE).astype(bf16)

    h1_s[0:8, :] = jnp.zeros((8, M), f32)
    h1_s[8 + S:16 + S, :] = jnp.zeros((8, M), f32)

    cp_ckv.wait()
    cp_wk0.wait()
    k_proj(0, 0)
    cp_wv0.wait()
    v_proj(0, 0)
    cp_c.wait()
    cp_wma.wait()
    cp_wq0.wait()
    mod = _modulation(c_s, wmod_a[...])
    sa = mod[:, 0:M]
    ca1 = 1.0 + mod[:, M:2 * M]
    _relayout(wq_raw, 0, M, 0, wq_s)
    def ln_rows(r0):
        xi = x_s[r0:r0 + LC, :].astype(f32)
        h_s[r0:r0 + LC, :] = (_layernorm(xi) * ca1 + sa).astype(bf16)

    for cp, (a, b) in zip(cp_x, xb):
        cp.wait()
        starts = list(range(a, b, LC))
        ln_rows(starts[0])
        for i, r0 in enumerate(starts):
            if i + 1 < len(starts):
                ln_rows(starts[i + 1])
            q_s[r0:r0 + LC, :] = (_dot(h_s[r0:r0 + LC, :], wq_s[...]) * QSCALE).astype(bf16)

    def group(g, carry):
        @pl.when(g == 2)
        def _():
            for cp in cp_later:
                cp.wait()

        @pl.when(g == 8)
        def _():
            for cp in cp_last:
                cp.wait()

        block = (g + 1) // 4
        pair = (g + 1) % 4
        _relayout(wk_raw, block, DC, pair, wk_s)

        def k_rows(r0):
            k_s[r0:r0 + KC, :] = _dot(ckv_s[r0:r0 + KC, :], wk_s[...]).astype(bf16)

        _attention_group(g, q_s, k_s, v_s, ctx_s, [functools.partial(k_rows, r0) for r0 in range(0, S, KC)])
        q_proj(block, pair)
        v_proj(block, pair)
        return carry

    lax.fori_loop(0, NG - 1, group, 0)
    _attention_group(NG - 1, q_s, k_s, v_s, ctx_s)

    _tail(x_s, ctx_s, wo_s, w1_s, w2_s, w3_s, w4_s, c_s, wmod_b, h1_s, out_s, o_hbm, osem)


@jax.jit
def pallas_adaLN_cond__compressed_kv_cla__mixer_s_mlp__prompt_kernel(
    A_x: jax.Array,
    A_c_kv: jax.Array,
    A_w_q: jax.Array,
    A_w_uk: jax.Array,
    A_w_uv: jax.Array,
    A_w_o: jax.Array,
    B_x: jax.Array,
    B_w1: jax.Array,
    B_w2: jax.Array,
    B_w3: jax.Array,
    B_w4: jax.Array,
    c: jax.Array,
    w_mod: jax.Array,
):
    del B_x
    x = A_x.reshape(S, M)
    ckv = A_c_kv.reshape(S, DC)
    wo = A_w_o.reshape(H * D, M)

    any_spec = pl.BlockSpec(memory_space=pl.ANY)
    scratch = [
        pltpu.VMEM((S, M), bf16),
        pltpu.VMEM((S // 2, DC), jnp.uint32),
        pltpu.VMEM((4, M, 8, D), jnp.uint32),
        pltpu.VMEM((4, DC, 8, D), jnp.uint32),
        pltpu.VMEM((4, DC, 8, D), jnp.uint32),
        pltpu.VMEM((H * D // 2, M), jnp.uint32),
        pltpu.VMEM((M // 2, M), jnp.uint32),
        pltpu.VMEM((M // 2, M), jnp.uint32),
        pltpu.VMEM((F // 2, M), jnp.uint32),
        pltpu.VMEM((F // 2, M), jnp.uint32),
        pltpu.VMEM((1, M), bf16),
        pltpu.VMEM((M, 2 * M), bf16),
        pltpu.VMEM((M, 4 * M), bf16),
        pltpu.VMEM((S // 2, M), jnp.uint32),
        pltpu.VMEM((M // 2, G * D), jnp.uint32),
        pltpu.VMEM((DC // 2, G * D), jnp.uint32),
        pltpu.VMEM((DC // 2, G * D), jnp.uint32),
        pltpu.VMEM((S // 2, G * D), jnp.uint32),
        pltpu.VMEM((S // 2, G * D), jnp.uint32),
        pltpu.VMEM((S // 2, G * D), jnp.uint32),
        pltpu.VMEM((NG, S // 2, G * D), jnp.uint32),
        pltpu.VMEM((S + 16, M), f32),
        pltpu.VMEM((S, M), bf16),
        pltpu.SemaphoreType.DMA((22 + len(XS),)),
        pltpu.SemaphoreType.DMA((S // TC,)),
    ]
    out = pl.pallas_call(
        _kernel,
        out_shape=jax.ShapeDtypeStruct((S, M), A_x.dtype),
        in_specs=[any_spec] * 12,
        out_specs=any_spec,
        scratch_shapes=scratch,
        compiler_params=pltpu.CompilerParams(vmem_limit_bytes=126 * 1024 * 1024),
    )(x, ckv, A_w_q, A_w_uk, A_w_uv, wo, B_w1, B_w2, B_w3.T, B_w4, c, w_mod)
    return out.reshape(1, S, M)
```

```python
import functools
import math

import jax
import jax.numpy as jnp
from jax import lax
from jax.experimental import pallas as pl
from jax.experimental.pallas import tpu as pltpu

S = 2048
M = 640
H = 32
D = 128
DC = 512
F = 1728
G = 2
assert G == 2
NG = H // G
R = 128
TC = 256
TIE = 6
LA = 1
LC = 128
KC = 1024
XS = (256, 768, 1280)
EPS = 1e-5
NEG = -1e9
QSCALE = float(D ** -0.5 * math.log2(math.e))

f32 = jnp.float32
bf16 = jnp.bfloat16
_NT = (((1,), (1,)), ((), ()))


def _dot(a, b):
    return jnp.dot(a, b, preferred_element_type=f32)


def _recip(x):
    r = pltpu.reciprocal(x, approx=True)
    r = r * (2.0 - x * r)
    return r * (2.0 - x * r)


def _layernorm(x):
    mu = jnp.mean(x, axis=-1, keepdims=True)
    xc = x - mu
    var = jnp.mean(xc * xc, axis=-1, keepdims=True)
    return xc * lax.rsqrt(var + EPS)


def _gelu(x):
    c = math.sqrt(2.0 / math.pi)
    return 0.5 * x * (1.0 + jnp.tanh(c * (x + 0.044715 * (x * x * x))))


def _relayout(w_raw, block, kdim, pair, dst_ref):
    w = w_raw.at[block].reshape(kdim * 8, D)
    for p in range(G // 2):
        x = w[pl.ds(pair + p, kdim, stride=8), :]
        lo = pltpu.bitcast(x << 16, f32).astype(bf16)
        hi = pltpu.bitcast(x & jnp.uint32(0xFFFF0000), f32).astype(bf16)
        dst_ref[:, (2 * p) * D:(2 * p + 1) * D] = lo
        dst_ref[:, (2 * p + 1) * D:(2 * p + 2) * D] = hi


def _attention_group(g, q_s, k_s, v_s, ctx_s, fillers=()):
    nstrip = S // R
    items = [(u, i) for u in range(G) for i in range(nstrip - 1, -1, -1)]
    n = len(items)
    st = {}
    inv = {}
    row = lax.broadcasted_iota(jnp.int32, (R, R), 0)
    col = lax.broadcasted_iota(jnp.int32, (R, R), 1)
    causal = col <= row

    def scores(t):
        u, i = items[t]
        e = (i + 1) * R
        q = q_s[i * R:(i + 1) * R, u * D:(u + 1) * D]
        s = lax.dot_general(q, k_s[0:e, u * D:(u + 1) * D], _NT, preferred_element_type=f32)
        tiles = [s[:, j * 128:(j + 1) * 128] for j in range(i)]
        tiles.append(jnp.where(causal, s[:, e - R:e], NEG))
        st[t] = {"tiles": tiles}

    def rowmax(t):
        d = st[t]
        m = d["tiles"][0]
        for x in d["tiles"][1:]:
            m = jnp.maximum(m, x)
        mm = jnp.max(m, axis=1, keepdims=True)
        if (t - TIE) in inv:
            mm = mm + 0.0 * inv.pop(t - TIE)
        d["m"] = mm

    def pv(t):
        u, i = items[t]
        d = st[t]
        e = (i + 1) * R
        ps = [jnp.exp2(x - d["m"]) for x in d["tiles"]]
        l = ps[0]
        for x in ps[1:]:
            l = l + x
        d["inv"] = _recip(jnp.sum(l, axis=1, keepdims=True))
        inv[t] = d["inv"]
        p = jnp.concatenate(ps, axis=1).astype(bf16)
        d["o"] = _dot(p, v_s[0:e, u * D:(u + 1) * D])

    def finish(t):
        u, i = items[t]
        d = st.pop(t)
        ctx_s[g, i * R:(i + 1) * R, u * D:(u + 1) * D] = (d["o"] * d["inv"]).astype(bf16)

    fillers = list(fillers)
    for t in range(-LA, n + 1):
        if 0 <= t + LA < n:
            scores(t + LA)
        if t + LA >= n - 1 and fillers:
            fillers.pop(0)()
        if 0 <= t + LA - 1 < n:
            rowmax(t + LA - 1)
        if 0 <= t < n:
            pv(t)
        if 0 <= t - 1 < n:
            finish(t - 1)
    for f in fillers:
        f()


def _tail(x_s, ctx_s, wo_s, w1_s, w2_s, w3_s, w4_s, c_s, wmod_s, h1_s, out_s, o_hbm, osem):
    n = S // TC
    PR = 16
    st = {}
    mod = _modulation(c_s, wmod_s[...])
    ga = mod[:, 0:M]
    sb = mod[:, M:2 * M]
    cb1 = 1.0 + mod[:, 2 * M:3 * M]
    gb = mod[:, 3 * M:4 * M]
    lane = lax.broadcasted_iota(jnp.int32, (1, 128), 1)
    out_copies = []
    pending = []

    def run_pending(k):
        for _ in range(min(k, len(pending))):
            pending.pop(0)()

    def rows(t):
        return slice(t * TC, (t + 1) * TC)

    def oproj(t):
        accs = []
        for c0 in range(0, M, 128):
            acc = None
            for g in range(0, NG, 2):
                lhs = jnp.concatenate([ctx_s[g + j, rows(t), :] for j in range(2)], axis=1)
                part = _dot(lhs, wo_s[g * G * D:(g + 2) * G * D, c0:c0 + 128])
                acc = part if acc is None else acc + part
            accs.append(acc)
            run_pending(8)
        acc = jnp.concatenate(accs, axis=1)
        d = st[t] = {"x1": [], "h": [], "n1": []}

        def piece(j):
            r = slice(j * PR, (j + 1) * PR)
            x1 = x_s[t * TC + j * PR:t * TC + (j + 1) * PR, :].astype(f32) + ga * acc[r]
            h = _layernorm(x1) * cb1 + sb
            d["x1"].append(x1)
            d["h"].append(h)
            d["n1"].append(_layernorm(h).astype(bf16))

        pending.extend(functools.partial(piece, j) for j in range(TC // PR))

    def mm1(t):
        run_pending(len(pending))
        d = st[t]
        h1_s[8 + t * TC:8 + (t + 1) * TC, :] = _gelu(_dot(jnp.concatenate(d.pop("n1"), axis=0), w1_s[...]))

    def mm2(t):
        d = st[t]
        r0 = 8 + t * TC

        def ld(shift, tile):
            return h1_s[r0 + shift:r0 + shift + TC, tile * 128:(tile + 1) * 128]

        c = M // 4
        g = jnp.concatenate([
            ld(-1, 0),
            jnp.where(lane < c - 128, ld(-1, 1), ld(1, 1)),
            jnp.where(lane < 2 * c - 256, ld(1, 2), ld(-2, 2)),
            jnp.where(lane < 3 * c - 384, ld(-2, 3), ld(2, 3)),
            ld(2, 4),
        ], axis=1).astype(bf16)
        hs = _dot(g, w2_s[...])
        d["u"] = []
        d["n2"] = []

        def piece(j):
            u = d["h"][j] + hs[j * PR:(j + 1) * PR]
            d["u"].append(u)
            d["n2"].append(_layernorm(u).astype(bf16))

        pending.extend(functools.partial(piece, j) for j in range(TC // PR))

    def mm3(t):
        d = st[t]
        while len(d["n2"]) < TC // PR:
            run_pending(1)
        a = lax.dot_general(jnp.concatenate(d.pop("n2"), axis=0), w3_s[...], _NT, preferred_element_type=f32)
        d["a"] = _gelu(a).astype(bf16)

    def mm4(t):
        d = st.pop(t)
        y = jnp.concatenate(d["u"], axis=0) + _dot(d["a"], w4_s[...])
        out_s[rows(t), :] = (jnp.concatenate(d["x1"], axis=0) + gb * y).astype(out_s.dtype)
        cp = pltpu.make_async_copy(out_s.at[rows(t), :], o_hbm.at[rows(t), :], osem.at[t])
        cp.start()
        out_copies.append(cp)

    for t in range(-2, n + 1):
        if 0 <= t + 2 < n:
            oproj(t + 2)
        if 0 <= t - 1 < n:
            mm3(t - 1)
        if 0 <= t + 1 < n:
            mm1(t + 1)
        if 0 <= t - 1 < n:
            mm4(t - 1)
        if 0 <= t < n:
            mm2(t)
    for cp in out_copies:
        cp.wait()


def _modulation(c_s, wmod):
    cv = c_s[...].astype(f32)
    sc = (cv * jax.nn.sigmoid(cv)).astype(bf16)
    return _dot(jnp.broadcast_to(sc, (16, M)), wmod)[0:1]


def _kernel(x_hbm, ckv_hbm, wq_hbm, wk_hbm, wv_hbm, wo_hbm, w1_hbm, w2_hbm, w3_hbm, w4_hbm, c_hbm, wmod_hbm,
            o_hbm,
            x_s, ckv_s, wq_raw, wk_raw, wv_raw, wo_s, w1_s, w2_s, w3_s, w4_s, c_s, wmod_a, wmod_b,
            h_s, wq_s, wk_s, wv_s, q_s, k_s, v_s, ctx_s, h1_s, out_s, sems, osem):
    u32 = jnp.uint32
    wq32, wk32, wv32 = (w.bitcast(u32) for w in (wq_hbm, wk_hbm, wv_hbm))
    xb = list(zip((0,) + XS, XS + (S,)))
    first = [
        (ckv_hbm.bitcast(u32), ckv_s),
        (wk32.at[:, 0:4, :], wk_raw.at[0, :, 0:4, :]),
        (wv32.at[:, 0:4, :], wv_raw.at[0, :, 0:4, :]),
        (c_hbm, c_s),
        (wmod_hbm.at[:, 0:2 * M], wmod_a),
        (wq32.at[:, 0:4, :], wq_raw.at[0, :, 0:4, :]),
    ] + [(x_hbm.at[a:b, :], x_s.at[a:b, :]) for a, b in xb]
    later = [(w32.at[:, 4 * q:4 * q + 4, :], raw.at[q, :, 0:4, :])
             for q in range(1, 4) for w32, raw in ((wk32, wk_raw), (wq32, wq_raw), (wv32, wv_raw))]
    last = [
        (wo_hbm.bitcast(u32), wo_s),
        (wmod_hbm.at[:, 2 * M:6 * M], wmod_b),
        (w1_hbm.bitcast(u32), w1_s),
        (w2_hbm.bitcast(u32), w2_s),
        (w3_hbm.bitcast(u32), w3_s),
        (w4_hbm.bitcast(u32), w4_s),
    ]
    copies = [pltpu.make_async_copy(src, dst, sems.at[i]) for i, (src, dst) in enumerate(first + later + last)]
    for cp in copies:
        cp.start()
    cp_ckv, cp_wk0, cp_wv0, cp_c, cp_wma, cp_wq0 = copies[:6]
    cp_x = copies[6:len(first)]
    cp_later = copies[len(first):len(first) + len(later)]
    cp_last = copies[len(first) + len(later):]
    ckv_s, wo_s, w1_s, w2_s, w3_s, w4_s, h_s, wq_s, wk_s, wv_s, q_s, k_s, v_s, ctx_s = (
        r.bitcast(bf16) for r in (ckv_s, wo_s, w1_s, w2_s, w3_s, w4_s, h_s, wq_s, wk_s, wv_s, q_s, k_s, v_s, ctx_s))

    def k_proj(block, pair):
        _relayout(wk_raw, block, DC, pair, wk_s)
        k_s[...] = _dot(ckv_s[...], wk_s[...]).astype(bf16)

    def v_proj(block, pair):
        _relayout(wv_raw, block, DC, pair, wv_s)
        v_s[...] = _dot(ckv_s[...], wv_s[...]).astype(bf16)

    def q_proj(block, pair):
        _relayout(wq_raw, block, M, pair, wq_s)
        q_s[...] = (_dot(h_s[...], wq_s[...]) * QSCALE).astype(bf16)

    h1_s[0:8, :] = jnp.zeros((8, M), f32)
    h1_s[8 + S:16 + S, :] = jnp.zeros((8, M), f32)

    cp_ckv.wait()
    cp_wk0.wait()
    k_proj(0, 0)
    cp_wv0.wait()
    v_proj(0, 0)
    cp_c.wait()
    cp_wma.wait()
    cp_wq0.wait()
    mod = _modulation(c_s, wmod_a[...])
    sa = mod[:, 0:M]
    ca1 = 1.0 + mod[:, M:2 * M]
    _relayout(wq_raw, 0, M, 0, wq_s)

    def ln_rows(r0):
        xi = x_s[r0:r0 + LC, :].astype(f32)
        h_s[r0:r0 + LC, :] = (_layernorm(xi) * ca1 + sa).astype(bf16)

    starts = list(range(0, S, LC))
    waits = {a: cp for cp, (a, _) in zip(cp_x, xb)}
    for i in range(len(starts) + 1):
        if i < len(starts):
            if starts[i] in waits:
                waits[starts[i]].wait()
            ln_rows(starts[i])
        if i > 0:
            r0 = starts[i - 1]
            q_s[r0:r0 + LC, :] = (_dot(h_s[r0:r0 + LC, :], wq_s[...]) * QSCALE).astype(bf16)

    def group(g, carry):
        @pl.when(g == 2)
        def _():
            for cp in cp_later:
                cp.wait()

        @pl.when(g == 8)
        def _():
            for cp in cp_last:
                cp.wait()

        block = (g + 1) // 4
        pair = (g + 1) % 4
        _relayout(wk_raw, block, DC, pair, wk_s)

        def k_rows(r0):
            k_s[r0:r0 + KC, :] = _dot(ckv_s[r0:r0 + KC, :], wk_s[...]).astype(bf16)

        _attention_group(g, q_s, k_s, v_s, ctx_s, [functools.partial(k_rows, r0) for r0 in range(0, S, KC)])
        q_proj(block, pair)
        v_proj(block, pair)
        return carry

    lax.fori_loop(0, NG - 1, group, 0)
    _attention_group(NG - 1, q_s, k_s, v_s, ctx_s)

    _tail(x_s, ctx_s, wo_s, w1_s, w2_s, w3_s, w4_s, c_s, wmod_b, h1_s, out_s, o_hbm, osem)


@jax.jit
def pallas_adaLN_cond__compressed_kv_cla__mixer_s_mlp__prompt_kernel(
    A_x: jax.Array,
    A_c_kv: jax.Array,
    A_w_q: jax.Array,
    A_w_uk: jax.Array,
    A_w_uv: jax.Array,
    A_w_o: jax.Array,
    B_x: jax.Array,
    B_w1: jax.Array,
    B_w2: jax.Array,
    B_w3: jax.Array,
    B_w4: jax.Array,
    c: jax.Array,
    w_mod: jax.Array,
):
    del B_x
    x = A_x.reshape(S, M)
    ckv = A_c_kv.reshape(S, DC)
    wo = A_w_o.reshape(H * D, M)

    any_spec = pl.BlockSpec(memory_space=pl.ANY)
    scratch = [
        pltpu.VMEM((S, M), bf16),
        pltpu.VMEM((S // 2, DC), jnp.uint32),
        pltpu.VMEM((4, M, 8, D), jnp.uint32),
        pltpu.VMEM((4, DC, 8, D), jnp.uint32),
        pltpu.VMEM((4, DC, 8, D), jnp.uint32),
        pltpu.VMEM((H * D // 2, M), jnp.uint32),
        pltpu.VMEM((M // 2, M), jnp.uint32),
        pltpu.VMEM((M // 2, M), jnp.uint32),
        pltpu.VMEM((F // 2, M), jnp.uint32),
        pltpu.VMEM((F // 2, M), jnp.uint32),
        pltpu.VMEM((1, M), bf16),
        pltpu.VMEM((M, 2 * M), bf16),
        pltpu.VMEM((M, 4 * M), bf16),
        pltpu.VMEM((S // 2, M), jnp.uint32),
        pltpu.VMEM((M // 2, G * D), jnp.uint32),
        pltpu.VMEM((DC // 2, G * D), jnp.uint32),
        pltpu.VMEM((DC // 2, G * D), jnp.uint32),
        pltpu.VMEM((S // 2, G * D), jnp.uint32),
        pltpu.VMEM((S // 2, G * D), jnp.uint32),
        pltpu.VMEM((S // 2, G * D), jnp.uint32),
        pltpu.VMEM((NG, S // 2, G * D), jnp.uint32),
        pltpu.VMEM((S + 16, M), f32),
        pltpu.VMEM((S, M), bf16),
        pltpu.SemaphoreType.DMA((22 + len(XS),)),
        pltpu.SemaphoreType.DMA((S // TC,)),
    ]
    out = pl.pallas_call(
        _kernel,
        out_shape=jax.ShapeDtypeStruct((S, M), A_x.dtype),
        in_specs=[any_spec] * 12,
        out_specs=any_spec,
        scratch_shapes=scratch,
        compiler_params=pltpu.CompilerParams(vmem_limit_bytes=126 * 1024 * 1024),
    )(x, ckv, A_w_q, A_w_uk, A_w_uv, wo, B_w1, B_w2, B_w3.T, B_w4, c, w_mod)
    return out.reshape(1, S, M)
```

```python
import functools
import math

import jax
import jax.numpy as jnp
from jax import lax
from jax.experimental import pallas as pl
from jax.experimental.pallas import tpu as pltpu

S = 2048
M = 640
H = 32
D = 128
DC = 512
F = 1728
G = 2
assert G == 2
NG = H // G
R = 128
TC = 256
TIE = 6
LA = 1
LC = 128
KC = 1024
XS = (256, 768, 1280)
EPS = 1e-5
NEG = -1e9
QSCALE = float(D ** -0.5 * math.log2(math.e))

f32 = jnp.float32
bf16 = jnp.bfloat16
_NT = (((1,), (1,)), ((), ()))


def _dot(a, b):
    return jnp.dot(a, b, preferred_element_type=f32)


def _recip(x):
    r = pltpu.reciprocal(x, approx=True)
    r = r * (2.0 - x * r)
    return r * (2.0 - x * r)


def _layernorm(x):
    mu = jnp.mean(x, axis=-1, keepdims=True)
    xc = x - mu
    var = jnp.mean(xc * xc, axis=-1, keepdims=True)
    return xc * lax.rsqrt(var + EPS)


def _gelu(x):
    c = math.sqrt(2.0 / math.pi)
    return 0.5 * x * (1.0 + jnp.tanh(c * (x + 0.044715 * (x * x * x))))


def _relayout(w_raw, block, kdim, pair, dst_ref):
    w = w_raw.at[block].reshape(kdim * 8, D)
    for p in range(G // 2):
        x = w[pl.ds(pair + p, kdim, stride=8), :]
        lo = pltpu.bitcast(x << 16, f32).astype(bf16)
        hi = pltpu.bitcast(x & jnp.uint32(0xFFFF0000), f32).astype(bf16)
        dst_ref[:, (2 * p) * D:(2 * p + 1) * D] = lo
        dst_ref[:, (2 * p + 1) * D:(2 * p + 2) * D] = hi


def _attention_group(g, q_s, k_s, v_s, ctx_s, fillers=()):
    nstrip = S // R
    items = [(u, i) for u in range(G) for i in range(nstrip - 1, -1, -1)]
    n = len(items)
    st = {}
    inv = {}
    row = lax.broadcasted_iota(jnp.int32, (R, R), 0)
    col = lax.broadcasted_iota(jnp.int32, (R, R), 1)
    causal = col <= row

    def scores(t):
        u, i = items[t]
        e = (i + 1) * R
        q = q_s[i * R:(i + 1) * R, u * D:(u + 1) * D]
        s = lax.dot_general(q, k_s[0:e, u * D:(u + 1) * D], _NT, preferred_element_type=f32)
        tiles = [s[:, j * 128:(j + 1) * 128] for j in range(i)]
        tiles.append(jnp.where(causal, s[:, e - R:e], NEG))
        st[t] = {"tiles": tiles}

    def rowmax(t):
        d = st[t]
        m = d["tiles"][0]
        for x in d["tiles"][1:]:
            m = jnp.maximum(m, x)
        mm = jnp.max(m, axis=1, keepdims=True)
        if (t - TIE) in inv:
            mm = mm + 0.0 * inv.pop(t - TIE)
        d["m"] = mm

    def pv(t):
        u, i = items[t]
        d = st[t]
        e = (i + 1) * R
        ps = [jnp.exp2(x - d["m"]) for x in d["tiles"]]
        l = ps[0]
        for x in ps[1:]:
            l = l + x
        d["inv"] = _recip(jnp.sum(l, axis=1, keepdims=True))
        inv[t] = d["inv"]
        p = jnp.concatenate(ps, axis=1).astype(bf16)
        d["o"] = _dot(p, v_s[0:e, u * D:(u + 1) * D])

    def finish(t):
        u, i = items[t]
        d = st.pop(t)
        ctx_s[g, i * R:(i + 1) * R, u * D:(u + 1) * D] = (d["o"] * d["inv"]).astype(bf16)

    fillers = list(fillers)
    for t in range(-LA, n + 1):
        if 0 <= t + LA < n:
            scores(t + LA)
        if t + LA >= n - 1 and fillers:
            fillers.pop(0)()
        if 0 <= t + LA - 1 < n:
            rowmax(t + LA - 1)
        if 0 <= t < n:
            pv(t)
        if 0 <= t - 1 < n:
            finish(t - 1)
    for f in fillers:
        f()


def _tail(x_s, ctx_s, wo_s, w1_s, w2_s, w3_s, w4_s, c_s, wmod_s, h1_s, out_s, o_hbm, osem):
    n = S // TC
    PR = 16
    st = {}
    mod = _modulation(c_s, wmod_s[...])
    ga = mod[:, 0:M]
    sb = mod[:, M:2 * M]
    cb1 = 1.0 + mod[:, 2 * M:3 * M]
    gb = mod[:, 3 * M:4 * M]
    lane = lax.broadcasted_iota(jnp.int32, (1, 128), 1)
    out_copies = []
    pending = []

    def run_pending(k):
        for _ in range(min(k, len(pending))):
            pending.pop(0)()

    def rows(t):
        return slice(t * TC, (t + 1) * TC)

    def oproj(t):
        accs = []
        for c0 in range(0, M, 128):
            acc = None
            for g in range(0, NG, 2):
                lhs = jnp.concatenate([ctx_s[g + j, rows(t), :] for j in range(2)], axis=1)
                part = _dot(lhs, wo_s[g * G * D:(g + 2) * G * D, c0:c0 + 128])
                acc = part if acc is None else acc + part
            accs.append(acc)
            run_pending(8)
        acc = jnp.concatenate(accs, axis=1)
        d = st[t] = {"x1": [], "h": [], "n1": []}

        def piece(j):
            r = slice(j * PR, (j + 1) * PR)
            x1 = x_s[t * TC + j * PR:t * TC + (j + 1) * PR, :].astype(f32) + ga * acc[r]
            h = _layernorm(x1) * cb1 + sb
            d["x1"].append(x1)
            d["h"].append(h)
            d["n1"].append(_layernorm(h).astype(bf16))

        pending.extend(functools.partial(piece, j) for j in range(TC // PR))

    def mm1(t):
        run_pending(len(pending))
        d = st[t]
        h1_s[8 + t * TC:8 + (t + 1) * TC, :] = _gelu(_dot(jnp.concatenate(d.pop("n1"), axis=0), w1_s[...]))

    def mm2(t):
        d = st[t]
        r0 = 8 + t * TC

        def ld(shift, tile):
            return h1_s[r0 + shift:r0 + shift + TC, tile * 128:(tile + 1) * 128]

        c = M // 4
        g = jnp.concatenate([
            ld(-1, 0),
            jnp.where(lane < c - 128, ld(-1, 1), ld(1, 1)),
            jnp.where(lane < 2 * c - 256, ld(1, 2), ld(-2, 2)),
            jnp.where(lane < 3 * c - 384, ld(-2, 3), ld(2, 3)),
            ld(2, 4),
        ], axis=1).astype(bf16)
        hs = _dot(g, w2_s[...])
        d["u"] = []
        d["n2"] = []

        def piece(j):
            u = d["h"][j] + hs[j * PR:(j + 1) * PR]
            d["u"].append(u)
            d["n2"].append(_layernorm(u).astype(bf16))

        pending.extend(functools.partial(piece, j) for j in range(TC // PR))

    def mm3(t):
        d = st[t]
        while len(d["n2"]) < TC // PR:
            run_pending(1)
        a = lax.dot_general(jnp.concatenate(d.pop("n2"), axis=0), w3_s[...], _NT, preferred_element_type=f32)
        d["a"] = _gelu(a).astype(bf16)

    def mm4(t):
        d = st.pop(t)
        u = jnp.concatenate(d["u"], axis=0)
        x1 = jnp.concatenate(d["x1"], axis=0)
        nsplit = 4 if t == n - 1 else 1
        hr = TC // nsplit
        for j in range(nsplit):
            r = slice(j * hr, (j + 1) * hr)
            orow = slice(t * TC + j * hr, t * TC + (j + 1) * hr)
            y = u[r] + _dot(d["a"][r], w4_s[...])
            out_s[orow, :] = (x1[r] + gb * y).astype(out_s.dtype)
            cp = pltpu.make_async_copy(out_s.at[orow, :], o_hbm.at[orow, :], osem.at[t + j])
            cp.start()
            out_copies.append(cp)

    for t in range(-2, n + 1):
        if 0 <= t + 2 < n:
            oproj(t + 2)
        if 0 <= t - 1 < n:
            mm3(t - 1)
        if 0 <= t + 1 < n:
            mm1(t + 1)
        if 0 <= t - 1 < n:
            mm4(t - 1)
        if 0 <= t < n:
            mm2(t)
    for cp in out_copies:
        cp.wait()


def _modulation(c_s, wmod):
    cv = c_s[...].astype(f32)
    sc = (cv * jax.nn.sigmoid(cv)).astype(bf16)
    return _dot(jnp.broadcast_to(sc, (16, M)), wmod)[0:1]


def _kernel(x_hbm, ckv_hbm, wq_hbm, wk_hbm, wv_hbm, wo_hbm, w1_hbm, w2_hbm, w3_hbm, w4_hbm, c_hbm, wmod_hbm,
            o_hbm,
            x_s, ckv_s, wq_raw, wk_raw, wv_raw, wo_s, w1_s, w2_s, w3_s, w4_s, c_s, wmod_a, wmod_b,
            h_s, wq_s, wk_s, wv_s, q_s, k_s, v_s, ctx_s, h1_s, out_s, sems, osem):
    u32 = jnp.uint32
    wq32, wk32, wv32 = (w.bitcast(u32) for w in (wq_hbm, wk_hbm, wv_hbm))
    xb = list(zip((0,) + XS, XS + (S,)))
    first = [
        (ckv_hbm.bitcast(u32), ckv_s),
        (wk32.at[:, 0:4, :], wk_raw.at[0, :, 0:4, :]),
        (wv32.at[:, 0:4, :], wv_raw.at[0, :, 0:4, :]),
        (c_hbm, c_s),
        (wmod_hbm.at[:, 0:2 * M], wmod_a),
        (wq32.at[:, 0:4, :], wq_raw.at[0, :, 0:4, :]),
    ] + [(x_hbm.at[a:b, :], x_s.at[a:b, :]) for a, b in xb]
    later = [(w32.at[:, 4 * q:4 * q + 4, :], raw.at[q, :, 0:4, :])
             for q in range(1, 4) for w32, raw in ((wk32, wk_raw), (wq32, wq_raw), (wv32, wv_raw))]
    last = [
        (wo_hbm.bitcast(u32), wo_s),
        (wmod_hbm.at[:, 2 * M:6 * M], wmod_b),
        (w1_hbm.bitcast(u32), w1_s),
        (w2_hbm.bitcast(u32), w2_s),
        (w3_hbm.bitcast(u32), w3_s),
        (w4_hbm.bitcast(u32), w4_s),
    ]
    copies = [pltpu.make_async_copy(src, dst, sems.at[i]) for i, (src, dst) in enumerate(first + later + last)]
    for cp in copies:
        cp.start()
    cp_ckv, cp_wk0, cp_wv0, cp_c, cp_wma, cp_wq0 = copies[:6]
    cp_x = copies[6:len(first)]
    cp_later = copies[len(first):len(first) + len(later)]
    cp_last = copies[len(first) + len(later):]
    ckv_s, wo_s, w1_s, w2_s, w3_s, w4_s, h_s, wq_s, wk_s, wv_s, q_s, k_s, v_s, ctx_s = (
        r.bitcast(bf16) for r in (ckv_s, wo_s, w1_s, w2_s, w3_s, w4_s, h_s, wq_s, wk_s, wv_s, q_s, k_s, v_s, ctx_s))

    def k_proj(block, pair):
        _relayout(wk_raw, block, DC, pair, wk_s)
        k_s[...] = _dot(ckv_s[...], wk_s[...]).astype(bf16)

    def v_proj(block, pair):
        _relayout(wv_raw, block, DC, pair, wv_s)
        v_s[...] = _dot(ckv_s[...], wv_s[...]).astype(bf16)

    def q_proj(block, pair):
        _relayout(wq_raw, block, M, pair, wq_s)
        q_s[...] = (_dot(h_s[...], wq_s[...]) * QSCALE).astype(bf16)

    h1_s[0:8, :] = jnp.zeros((8, M), f32)
    h1_s[8 + S:16 + S, :] = jnp.zeros((8, M), f32)

    cp_ckv.wait()
    cp_wk0.wait()
    k_proj(0, 0)
    cp_wv0.wait()
    v_proj(0, 0)
    cp_c.wait()
    cp_wma.wait()
    cp_wq0.wait()
    mod = _modulation(c_s, wmod_a[...])
    sa = mod[:, 0:M]
    ca1 = 1.0 + mod[:, M:2 * M]
    _relayout(wq_raw, 0, M, 0, wq_s)

    def ln_rows(r0):
        xi = x_s[r0:r0 + LC, :].astype(f32)
        h_s[r0:r0 + LC, :] = (_layernorm(xi) * ca1 + sa).astype(bf16)

    starts = list(range(0, S, LC))
    waits = {a: cp for cp, (a, _) in zip(cp_x, xb)}
    for i in range(len(starts) + 1):
        if i < len(starts):
            if starts[i] in waits:
                waits[starts[i]].wait()
            ln_rows(starts[i])
        if i > 0:
            r0 = starts[i - 1]
            q_s[r0:r0 + LC, :] = (_dot(h_s[r0:r0 + LC, :], wq_s[...]) * QSCALE).astype(bf16)

    def group(g, carry):
        @pl.when(g == 2)
        def _():
            for cp in cp_later:
                cp.wait()

        @pl.when(g == 8)
        def _():
            for cp in cp_last:
                cp.wait()

        block = (g + 1) // 4
        pair = (g + 1) % 4
        _relayout(wk_raw, block, DC, pair, wk_s)

        def k_rows(r0):
            k_s[r0:r0 + KC, :] = _dot(ckv_s[r0:r0 + KC, :], wk_s[...]).astype(bf16)

        _attention_group(g, q_s, k_s, v_s, ctx_s, [functools.partial(k_rows, r0) for r0 in range(0, S, KC)])
        q_proj(block, pair)
        v_proj(block, pair)
        return carry

    lax.fori_loop(0, NG - 1, group, 0)
    _attention_group(NG - 1, q_s, k_s, v_s, ctx_s)

    _tail(x_s, ctx_s, wo_s, w1_s, w2_s, w3_s, w4_s, c_s, wmod_b, h1_s, out_s, o_hbm, osem)


@jax.jit
def pallas_adaLN_cond__compressed_kv_cla__mixer_s_mlp__prompt_kernel(
    A_x: jax.Array,
    A_c_kv: jax.Array,
    A_w_q: jax.Array,
    A_w_uk: jax.Array,
    A_w_uv: jax.Array,
    A_w_o: jax.Array,
    B_x: jax.Array,
    B_w1: jax.Array,
    B_w2: jax.Array,
    B_w3: jax.Array,
    B_w4: jax.Array,
    c: jax.Array,
    w_mod: jax.Array,
):
    del B_x
    x = A_x.reshape(S, M)
    ckv = A_c_kv.reshape(S, DC)
    wo = A_w_o.reshape(H * D, M)

    any_spec = pl.BlockSpec(memory_space=pl.ANY)
    scratch = [
        pltpu.VMEM((S, M), bf16),
        pltpu.VMEM((S // 2, DC), jnp.uint32),
        pltpu.VMEM((4, M, 8, D), jnp.uint32),
        pltpu.VMEM((4, DC, 8, D), jnp.uint32),
        pltpu.VMEM((4, DC, 8, D), jnp.uint32),
        pltpu.VMEM((H * D // 2, M), jnp.uint32),
        pltpu.VMEM((M // 2, M), jnp.uint32),
        pltpu.VMEM((M // 2, M), jnp.uint32),
        pltpu.VMEM((F // 2, M), jnp.uint32),
        pltpu.VMEM((F // 2, M), jnp.uint32),
        pltpu.VMEM((1, M), bf16),
        pltpu.VMEM((M, 2 * M), bf16),
        pltpu.VMEM((M, 4 * M), bf16),
        pltpu.VMEM((S // 2, M), jnp.uint32),
        pltpu.VMEM((M // 2, G * D), jnp.uint32),
        pltpu.VMEM((DC // 2, G * D), jnp.uint32),
        pltpu.VMEM((DC // 2, G * D), jnp.uint32),
        pltpu.VMEM((S // 2, G * D), jnp.uint32),
        pltpu.VMEM((S // 2, G * D), jnp.uint32),
        pltpu.VMEM((S // 2, G * D), jnp.uint32),
        pltpu.VMEM((NG, S // 2, G * D), jnp.uint32),
        pltpu.VMEM((S + 16, M), f32),
        pltpu.VMEM((S, M), bf16),
        pltpu.SemaphoreType.DMA((22 + len(XS),)),
        pltpu.SemaphoreType.DMA((S // TC + 3,)),
    ]
    out = pl.pallas_call(
        _kernel,
        out_shape=jax.ShapeDtypeStruct((S, M), A_x.dtype),
        in_specs=[any_spec] * 12,
        out_specs=any_spec,
        scratch_shapes=scratch,
        compiler_params=pltpu.CompilerParams(vmem_limit_bytes=126 * 1024 * 1024),
    )(x, ckv, A_w_q, A_w_uk, A_w_uv, wo, B_w1, B_w2, B_w3.T, B_w4, c, w_mod)
    return out.reshape(1, S, M)
```
